```python
import jax
import jax.numpy as jnp

def _softmax(x, axis=-1):
    return jax.nn.softmax(x, axis=axis)
def _gelu(x):
    return jax.nn.gelu(x, approximate=True)
def _silu(x):
    return jax.nn.silu(x)
def _sigmoid(x):
    return jax.nn.sigmoid(x)
def _layernorm(x, axis=-1, eps=1e-5):
    m = jnp.mean(x, axis=axis, keepdims=True)
    v = jnp.var(x, axis=axis, keepdims=True)
    return (x - m) / jnp.sqrt(v + eps)
def _scatter_add(tgt, idx, src, axis=0):
    return tgt.at[idx].add(src)
def _segment_sum(src, seg, n):
    return jax.ops.segment_sum(src, seg, n)
class _Rng:
    def __init__(self, key):
        self._k = key
    def _next(self):
        self._k, sub = jax.random.split(self._k)
        return sub
    def normal(self, shape):
        return jax.random.normal(self._next(), shape, dtype=jnp.bfloat16)
    def randint(self, lo, hi, shape):
        return jax.random.randint(self._next(), shape, lo, hi, dtype=jnp.int32)
    def uniform(self, shape, lo=0.0, hi=1.0):
        return jax.random.uniform(self._next(), shape, jnp.bfloat16, lo, hi)
    def permutation(self, n):
        return jax.random.permutation(self._next(), n)


kernel_name = 'interleave_layers__sliding_block__sliding_local_dilated__prompt'

def setup_inputs():
    _rng = _Rng(jax.random.key(int.from_bytes(__import__("os").urandom(4), "little")))
    _w = (lambda a: (lambda t: t.astype(jnp.bfloat16) if jnp.issubdtype(t.dtype, jnp.floating) else t)(jnp.asarray(a)))
    def _A_setup():
        B, S, D = 1, 2048, 1024
        return {
            "x": _w((lambda *s: _rng.normal(s) * 0.05)(B, S, D)),
            "wqkv": _w((lambda *s: _rng.normal(s) * 0.05)(D, 3 * D)),
            "wo": _w((lambda *s: _rng.normal(s) * 0.05)(D, D)),
        }
    _A_in = _A_setup()

    def _B_setup():
        B, S, D = 1, 2048, 1024
        return {
            "x": _w((lambda *s: _rng.normal(s) * 0.05)(B, S, D)),
            "wqkv": _w((lambda *s: _rng.normal(s) * 0.05)(D, 3 * D)),
            "wo": _w((lambda *s: _rng.normal(s) * 0.05)(D, D)),
        }
    _B_in = _B_setup()

    return {
        "A_x": _A_in["x"],
        "A_wqkv": _A_in["wqkv"],
        "A_wo": _A_in["wo"],
        "B_x": _B_in["x"],
        "B_wqkv": _B_in["wqkv"],
        "B_wo": _B_in["wo"],
    }

def reference(A_x, A_wqkv, A_wo, B_x, B_wqkv, B_wo):
    def _A_ref(x, wqkv, wo):
        B, S, D = x.shape
        H = 32; Dh = D // H; W = 256
        qkv = (lambda x, *d: x.transpose(*d))((x @ wqkv).reshape(B, S, 3, H, Dh), 2, 0, 3, 1, 4)
        q, k, v = qkv[0], qkv[1], qkv[2]
        scores = jnp.einsum("bhqd,bhkd->bhqk", q, k) * (Dh ** -0.5)
        idx = jnp.arange(S)
        mask = (idx[:, None] - idx[None, :] >= 0) & (idx[:, None] - idx[None, :] < W)
        scores = jnp.where(mask[None, None], scores, -1e9)
        p = _softmax(scores, axis=-1)
        o = jnp.einsum("bhqk,bhkd->bhqd", p, v)
        return (lambda x, *d: x.transpose(*d))(o, 0, 2, 1, 3).reshape(B, S, D) @ wo

    def _B_ref(x, wqkv, wo):
        B, S, D = x.shape
        H = 32; Dh = D // H
        W, dil = 8, 2
        qkv = (lambda x, *d: x.transpose(*d))((x @ wqkv).reshape(B, S, 3, H, Dh), 2, 0, 3, 1, 4)
        q, k, v = qkv[0], qkv[1], qkv[2]
        scale = Dh ** -0.5
        pos = jnp.arange(S)
        off = jnp.arange(W) * dil
        idx = pos[:, None] - off[None, :]
        mask = idx >= 0
        idx_c = jnp.where(mask, idx, 0).reshape(-1)
        kg = k[:, :, idx_c, :].reshape(B, H, S, W, Dh)
        vg = v[:, :, idx_c, :].reshape(B, H, S, W, Dh)
        logits = jnp.einsum("bhsd,bhswd->bhsw", q, kg) * scale
        logits = jnp.where(mask[None, None, :, :], logits, -1e9)
        attn = _softmax(logits, axis=-1)
        o = jnp.einsum("bhsw,bhswd->bhsd", attn, vg)
        return (lambda x, *d: x.transpose(*d))(o, 0, 2, 1, 3).reshape(B, S, D) @ wo

    x = A_x
    x = x + _A_ref(_layernorm(x, axis=-1), A_wqkv, A_wo)
    x = x + _B_ref(_layernorm(x, axis=-1), B_wqkv, B_wo)
    x = x + _A_ref(_layernorm(x, axis=-1), A_wqkv, A_wo)
    x = x + _B_ref(_layernorm(x, axis=-1), B_wqkv, B_wo)
    return x
```

```python
import functools
import math

import jax
import jax.numpy as jnp
from jax import lax
import jax.experimental.pallas as pl
import jax.experimental.pallas.tpu as pltpu

S = 2048
D = 1024
NG = 8
DH = 32
PAD = 256
R = 256
NB = S // R
EPS = 1e-5
NEG = -1e9
QSCALE = (DH ** -0.5) * math.log2(math.e)

_NT = (((1,), (1,)), ((), ()))


def _kernel(x_hbm, wqa_hbm, woa_hbm, wqb_hbm, wob_hbm, out_hbm,
            xres, xio, wq, wo, q_s, k_s, v_s, o_s, xn_s, sems):
    f32, bf16, i32 = jnp.float32, jnp.bfloat16, jnp.int32

    cp_x = pltpu.make_async_copy(x_hbm, xio, sems.at[0])
    cp_wqa = pltpu.make_async_copy(wqa_hbm, wq.at[0], sems.at[1])
    cp_woa = pltpu.make_async_copy(woa_hbm, wo.at[0], sems.at[2])
    cp_wqb = pltpu.make_async_copy(wqb_hbm, wq.at[1], sems.at[3])
    cp_wob = pltpu.make_async_copy(wob_hbm, wo.at[1], sems.at[4])
    cp_x.start()
    cp_wqa.start()
    cp_woa.start()
    cp_wqb.start()
    cp_wob.start()

    k_s[:, PAD - 64:PAD, :] = jnp.zeros((NG, 64, 128), bf16)
    v_s[:, PAD - 64:PAD, :] = jnp.zeros((NG, 64, 128), bf16)
    cp_x.wait()

    def cvt(i, c):
        r0 = pl.multiple_of(i * R, R)
        xres[pl.ds(r0, R), :] = xio[pl.ds(r0, R), :].astype(f32)
        return c
    lax.fori_loop(0, NB, cvt, 0)

    def lane_group(n):
        return lax.broadcasted_iota(i32, (n, 128), 1) // DH

    def stack_heads(q):
        n = q.shape[0]
        qi = pltpu.bitcast(q, i32)
        lg = lane_group(n // 2)
        parts = [pltpu.bitcast(jnp.where(lg == h, qi, 0), bf16) for h in range(4)]
        return jnp.concatenate(parts, axis=0)

    def unstack_heads(o, n):
        lg = lane_group(n)
        r = o[3 * n:4 * n]
        for h in (2, 1, 0):
            r = jnp.where(lg == h, o[h * n:(h + 1) * n], r)
        return r

    def causal_masks():
        lane = lax.broadcasted_iota(i32, (128, 128), 1)
        row = lax.broadcasted_iota(i32, (128, 128), 0)
        cm = lane <= row
        lane2 = lax.broadcasted_iota(i32, (64, 128), 1)
        row2 = lax.broadcasted_iota(i32, (64, 128), 0) * 2
        mlo = jnp.where(lane2 <= row2, 0x0000FFFF, 0)
        mhi = jnp.where(lane2 <= row2 + 1, -65536, 0)
        return cm, mlo | mhi

    def part_ln(blk, r):
        r32 = pl.multiple_of(r * 32, 32)
        x = xres[pl.ds(pl.multiple_of(blk * R + r32, 32), 32), :]
        m = jnp.mean(x, axis=-1, keepdims=True)
        xc = x - m
        v = jnp.mean(xc * xc, axis=-1, keepdims=True)
        xn_s[blk % 2, pl.ds(r32, 32), :] = (xc * lax.rsqrt(v + EPS)).astype(bf16)

    def part_qkv(wi, blk, g):
        r0 = pl.multiple_of(blk * R, R)
        xn = xn_s[blk % 2]
        for which in range(3):
            c0 = pl.multiple_of(g * 128 + which * D, 128)
            a = jnp.dot(xn, wq[wi, :, pl.ds(c0, 128)], preferred_element_type=f32)
            if which == 0:
                q_s[g, pl.ds(r0, R), :] = (a * QSCALE).astype(bf16)
            elif which == 1:
                k_s[g, pl.ds(r0 + PAD, R), :] = a.astype(bf16)
            else:
                v_s[g, pl.ds(r0 + PAD, R), :] = a.astype(bf16)

    def part_out(wi, blk, g, last):
        r0 = pl.multiple_of(blk * R, R)
        c0 = pl.multiple_of(g * 128, 128)
        o = jnp.concatenate([o_s[blk % 2, gg] for gg in range(NG)], axis=1)
        y = jnp.dot(o, wo[wi, :, pl.ds(c0, 128)], preferred_element_type=f32)
        y = y + xres[pl.ds(r0, R), pl.ds(c0, 128)]
        if last:
            xio[pl.ds(r0, R), pl.ds(c0, 128)] = y.astype(bf16)
        else:
            xres[pl.ds(r0, R), pl.ds(c0, 128)] = y

    def a_scores(g, blk, j, nkb):
        r0 = pl.multiple_of(blk * R + j * 128, 128)
        qs = stack_heads(q_s[g, pl.ds(r0, 128), :])
        k0 = pl.multiple_of(r0 + (3 - nkb) * 128, 128)
        kw = k_s[g, pl.ds(k0, nkb * 128), :]
        return lax.dot_general(qs, kw, _NT, preferred_element_type=f32)

    def a_softmax(s, nkb):
        cm, cmi = causal_masks()
        cm4 = jnp.concatenate([cm] * 4, axis=0)
        sd = s[:, (nkb - 1) * 128:]
        if nkb == 3:
            sm = jnp.where(cm4, sd, s[:, 0:128])
        else:
            sm = jnp.where(cm4, sd, NEG)
        if nkb >= 2:
            s1 = s[:, (nkb - 2) * 128:(nkb - 1) * 128]
            m = jnp.max(jnp.maximum(sm, s1), axis=-1, keepdims=True)
            pm = jnp.exp2(sm - m)
            p1 = jnp.exp2(s1 - m)
            l = jnp.sum(pm + p1, axis=-1, keepdims=True)
        else:
            m = jnp.max(sm, axis=-1, keepdims=True)
            pm = jnp.exp2(sm - m)
            l = jnp.sum(pm, axis=-1, keepdims=True)
        pmb = pm.astype(bf16)
        if nkb == 3:
            pmi = pltpu.bitcast(pmb, i32)
            cmi4 = jnp.concatenate([cmi] * 4, axis=0)
            p = jnp.concatenate([pltpu.bitcast(pmi & (~cmi4), bf16), p1.astype(bf16),
                                 pltpu.bitcast(pmi & cmi4, bf16)], axis=1)
        elif nkb == 2:
            p = jnp.concatenate([p1.astype(bf16), pmb], axis=1)
        else:
            p = pmb
        lsel = unstack_heads(jnp.broadcast_to(l, (512, 128)), 128)
        return p, 1.0 / lsel

    def a_values(g, blk, j, nkb, p, rl):
        r0 = pl.multiple_of(blk * R + j * 128, 128)
        k0 = pl.multiple_of(r0 + (3 - nkb) * 128, 128)
        vw = v_s[g, pl.ds(k0, nkb * 128), :]
        o = jnp.dot(p, vw, preferred_element_type=f32)
        o_s[blk % 2, g, j * 128:(j + 1) * 128, :] = (unstack_heads(o, 128) * rl).astype(bf16)

    def b_scores(g, blk, j):
        r0 = pl.multiple_of(blk * R + j * 64, 64)
        qs = stack_heads(q_s[g, pl.ds(r0, 64), :])
        k0 = pl.multiple_of(r0 + (PAD - 64), 64)
        kw = k_s[g, pl.ds(k0, 128), :]
        return lax.dot_general(qs, kw, _NT, preferred_element_type=f32)

    def b_softmax(s, blk, j):
        lane = lax.broadcasted_iota(i32, (64, 128), 1)
        row = lax.broadcasted_iota(i32, (64, 128), 0)
        dlt = row + 64 - lane
        ok = (dlt >= 0) & (dlt <= 14) & ((dlt & 1) == 0)
        if j == 0:
            ok = ok & (lane + blk * R >= 64)
        ok4 = jnp.concatenate([ok] * 4, axis=0)
        s = jnp.where(ok4, s, NEG)
        m = jnp.max(s, axis=-1, keepdims=True)
        p = jnp.exp2(s - m)
        l = jnp.sum(p, axis=-1, keepdims=True)
        lsel = unstack_heads(jnp.broadcast_to(l, (256, 128)), 64)
        return p.astype(bf16), 1.0 / lsel

    def b_values(g, blk, j, p, rl):
        r0 = pl.multiple_of(blk * R + j * 64, 64)
        k0 = pl.multiple_of(r0 + (PAD - 64), 64)
        vw = v_s[g, pl.ds(k0, 128), :]
        o = jnp.dot(p, vw, preferred_element_type=f32)
        o_s[blk % 2, g, j * 64:(j + 1) * 64, :] = (unstack_heads(o, 64) * rl).astype(bf16)

    def run_steps(layer, i_lo, i_hi, do_b, do_c, do_d, edge=False):
        typ = layer % 2
        last_layer = layer == 3

        def body(t, c):
            i = i_lo + t // NG
            g = t % NG
            if typ == 0:
                nkb = [(j + 1) if edge else 3 for j in range(2)]
                ss = [a_scores(g, i, j, nkb[j]) for j in range(2)]
            else:
                ss = [b_scores(g, i, j) for j in range(4)]
            if do_d:
                part_ln((i + 2) % NB, g)
            if typ == 0:
                ps = [a_softmax(ss[j], nkb[j]) for j in range(2)]
            else:
                ps = [b_softmax(ss[j], i, j) for j in range(4)]
            if do_c:
                if isinstance(i_lo, int) and i_lo >= 1:
                    part_out(typ, i - 1, g, last_layer)
                else:
                    part_out((layer + NB + (i - 1) // NB) % 2, (i + NB - 1) % NB, g, False)
            if typ == 0:
                for j in range(2):
                    a_values(g, i, j, nkb[j], *ps[j])
            else:
                for j in range(4):
                    b_values(g, i, j, *ps[j])
            if do_b:
                part_qkv((layer + (i + 1) // NB) % 2, (i + 1) % NB, g)
            return c
        lax.fori_loop(0, (i_hi - i_lo) * NG, body, 0)

    def out_dma(blk):
        r0 = pl.multiple_of(blk * R, R)
        return pltpu.make_async_copy(xio.at[pl.ds(r0, R), :], out_hbm.at[pl.ds(r0, R), :],
                                     sems.at[5])

    def pro_ln(t, c):
        part_ln(t // NG, t % NG)
        return c
    lax.fori_loop(0, 2 * NG, pro_ln, 0)
    cp_wqa.wait()

    def pro_qkv(g, c):
        part_qkv(0, 0, g)
        return c
    lax.fori_loop(0, NG, pro_qkv, 0)

    run_steps(0, 0, 1, True, False, True, edge=True)
    cp_woa.wait()
    cp_wqb.wait()
    run_steps(0, 1, NB, True, True, True)
    cp_wob.wait()
    run_steps(1, 0, NB, True, True, True)
    run_steps(2, 0, 1, True, True, True, edge=True)
    run_steps(2, 1, NB, True, True, True)
    run_steps(3, 0, 1, True, True, True)
    for i in range(1, NB - 1):
        run_steps(3, i, i + 1, True, True, i < NB - 2)
        out_dma(i - 1).start()
    run_steps(3, NB - 1, NB, False, True, False)
    out_dma(NB - 2).start()

    def epi(g, c):
        part_out(1, NB - 1, g, True)
        return c
    lax.fori_loop(0, NG, epi, 0)
    out_dma(NB - 1).start()
    pltpu.make_async_copy(xio, out_hbm, sems.at[5]).wait()


@jax.jit
def pallas_interleave_layers__sliding_block__sliding_local_dilated__prompt_kernel(
    A_x: jax.Array,
    A_wqkv: jax.Array,
    A_wo: jax.Array,
    B_x: jax.Array,
    B_wqkv: jax.Array,
    B_wo: jax.Array,
):
    del B_x
    bf16, f32 = jnp.bfloat16, jnp.float32
    any_spec = pl.BlockSpec(memory_space=pl.ANY)
    out = pl.pallas_call(
        _kernel,
        in_specs=[any_spec] * 5,
        out_specs=any_spec,
        out_shape=jax.ShapeDtypeStruct((S, D), bf16),
        scratch_shapes=[
            pltpu.VMEM((S, D), f32),
            pltpu.VMEM((S, D), bf16),
            pltpu.VMEM((2, D, 3 * D), bf16),
            pltpu.VMEM((2, D, D), bf16),
            pltpu.VMEM((NG, S, 128), bf16),
            pltpu.VMEM((NG, PAD + S, 128), bf16),
            pltpu.VMEM((NG, PAD + S, 128), bf16),
            pltpu.VMEM((2, NG, R, 128), bf16),
            pltpu.VMEM((2, R, D), bf16),
            pltpu.SemaphoreType.DMA((6,)),
        ],
        compiler_params=pltpu.CompilerParams(vmem_limit_bytes=100 * 1024 * 1024),
    )(A_x.reshape(S, D), A_wqkv, A_wo, B_wqkv, B_wo)
    return out.reshape(1, S, D)
```

```python
import functools
import math

import jax
import jax.numpy as jnp
from jax import lax
import jax.experimental.pallas as pl
import jax.experimental.pallas.tpu as pltpu

S = 2048
D = 1024
NG = 8
DH = 32
PAD = 256
R = 256
NB = S // R
NQ1 = 1
GU = 2
EPS = 1e-5
NEG = -1e9
QSCALE = (DH ** -0.5) * math.log2(math.e)

_NT = (((1,), (1,)), ((), ()))


def _kernel(x_hbm, wqa_hbm, woa_hbm, wqb_hbm, wob_hbm, out_hbm,
            xres, xio, wq, wo, q_s, k_s, v_s, o_s, xn_s, sems):
    f32, bf16, i32 = jnp.float32, jnp.bfloat16, jnp.int32

    cp_x0 = pltpu.make_async_copy(x_hbm.at[0:2 * R], xio.at[0:2 * R], sems.at[0])
    cp_x1 = pltpu.make_async_copy(x_hbm.at[2 * R:S], xio.at[2 * R:S], sems.at[1])
    cp_woa = pltpu.make_async_copy(woa_hbm, wo.at[0], sems.at[2])
    cp_wqb = pltpu.make_async_copy(wqb_hbm, wq.at[1], sems.at[3])
    cp_wob = pltpu.make_async_copy(wob_hbm, wo.at[1], sems.at[4])

    def cp_wqa(g):
        return [pltpu.make_async_copy(wqa_hbm.at[:, pl.ds(g * 128 + w * D, 128)],
                                      wq.at[0, :, pl.ds(g * 128 + w * D, 128)],
                                      sems.at[6 + g]) for w in range(3)]

    cp_x0.start()
    for cp in cp_wqa(0) + cp_wqa(1):
        cp.start()

    k_s[:, PAD - 32:PAD, :] = jnp.zeros((NG, 32, 128), bf16)
    v_s[:, PAD - 32:PAD, :] = jnp.zeros((NG, 32, 128), bf16)

    def cvt(i, c):
        r0 = pl.multiple_of(i * R, R)
        xres[pl.ds(r0, R), :] = xio[pl.ds(r0, R), :].astype(f32)
        return c

    def lane_group(n):
        return lax.broadcasted_iota(i32, (n, 128), 1) // DH

    def stack_heads(q):
        n = q.shape[0]
        qi = pltpu.bitcast(q, i32)
        lg = lane_group(n // 2)
        parts = [pltpu.bitcast(jnp.where(lg == h, qi, 0), bf16) for h in range(4)]
        return jnp.concatenate(parts, axis=0)

    def unstack_heads(o, n):
        lg = lane_group(n)
        r = o[3 * n:4 * n]
        for h in (2, 1, 0):
            r = jnp.where(lg == h, o[h * n:(h + 1) * n], r)
        return r

    def causal_masks():
        lane = lax.broadcasted_iota(i32, (128, 128), 1)
        row = lax.broadcasted_iota(i32, (128, 128), 0)
        cm = lane <= row
        lane2 = lax.broadcasted_iota(i32, (64, 128), 1)
        row2 = lax.broadcasted_iota(i32, (64, 128), 0) * 2
        mlo = jnp.where(lane2 <= row2, 0x0000FFFF, 0)
        mhi = jnp.where(lane2 <= row2 + 1, -65536, 0)
        return cm, mlo | mhi

    def part_ln(blk, r):
        r32 = pl.multiple_of(r * 32, 32)
        x = xres[pl.ds(pl.multiple_of(blk * R + r32, 32), 32), :]
        m = jnp.mean(x, axis=-1, keepdims=True)
        xc = x - m
        v = jnp.mean(xc * xc, axis=-1, keepdims=True)
        xn_s[blk % 2, pl.ds(r32, 32), :] = (xc * lax.rsqrt(v + EPS)).astype(bf16)

    def part_qkv(wi, blk, g):
        r0 = pl.multiple_of(blk * R, R)
        xn = xn_s[blk % 2]
        for which in range(3):
            c0 = pl.multiple_of(g * 128 + which * D, 128)
            a = jnp.dot(xn, wq[wi, :, pl.ds(c0, 128)], preferred_element_type=f32)
            if which == 0:
                q_s[g, pl.ds(r0, R), :] = (a * QSCALE).astype(bf16)
            elif which == 1:
                k_s[g, pl.ds(r0 + PAD, R), :] = a.astype(bf16)
            else:
                v_s[g, pl.ds(r0 + PAD, R), :] = a.astype(bf16)

    def part_out(wi, blk, g, last):
        r0 = pl.multiple_of(blk * R, R)
        c0 = pl.multiple_of(g * 128, 128)
        o = jnp.concatenate([o_s[blk % 2, gg] for gg in range(NG)], axis=1)
        y = jnp.dot(o, wo[wi, :, pl.ds(c0, 128)], preferred_element_type=f32)
        y = y + xres[pl.ds(r0, R), pl.ds(c0, 128)]
        if last:
            xio[pl.ds(r0, R), pl.ds(c0, 128)] = y.astype(bf16)
        else:
            xres[pl.ds(r0, R), pl.ds(c0, 128)] = y

    def seg_reduce(x, op, fill):
        lg = lane_group(x.shape[0])
        r = None
        for h in range(4):
            rh = op(jnp.where(lg == h, x, fill), axis=-1, keepdims=True)
            r = jnp.broadcast_to(rh, x.shape) if r is None else jnp.where(lg == h, rh, r)
        return r

    def tri_mask(n):
        kk = lax.broadcasted_iota(i32, (n, 128), 1) % DH
        return kk <= lax.broadcasted_iota(i32, (n, 128), 0)

    def tri_mask_packed(n):
        kk = lax.broadcasted_iota(i32, (n // 2, 128), 1) % DH
        row2 = lax.broadcasted_iota(i32, (n // 2, 128), 0) * 2
        return jnp.where(kk <= row2, 0x0000FFFF, 0) | jnp.where(kk <= row2 + 1, -65536, 0)

    def a_scores(g, blk, edge):
        r0 = pl.multiple_of(blk * R, R)
        q = q_s[g, pl.ds(r0, R), :]
        k0 = 8 if edge else 0
        kw = k_s[g, pl.ds(r0 + 32 * k0, 32 * (16 - k0)), :]
        ss = {}
        for kb in range(k0, 16):
            kbd = stack_heads(kw[32 * (kb - k0):32 * (kb - k0) + 32])
            qq = q[0:32 * kb + 32] if kb < 8 else q[32 * (kb - 8):R]
            ss[kb] = lax.dot_general(qq, kbd, _NT, preferred_element_type=f32)
        return ss

    def a_softmax(ss, edge):
        tri = tri_mask(32)
        t = {}
        for kb in range(8):
            for rb in range(8):
                if rb == kb:
                    old = NEG if edge else ss[kb][32 * kb:32 * kb + 32]
                    t[kb, rb] = jnp.where(tri, ss[kb + 8][0:32], old)
                elif rb > kb:
                    t[kb, rb] = ss[kb + 8][32 * (rb - kb):32 * (rb - kb) + 32]
                elif not edge:
                    t[kb, rb] = ss[kb][32 * rb:32 * rb + 32]
        trip = tri_mask_packed(32)
        pp, rl = {}, []
        for rb in range(8):
            ks = [kb for kb in range(8) if (kb, rb) in t]
            m = functools.reduce(jnp.maximum, [t[kb, rb] for kb in ks])
            m = seg_reduce(m, jnp.max, -jnp.inf)
            p = {kb: jnp.exp2(t[kb, rb] - m) for kb in ks}
            l = seg_reduce(functools.reduce(jnp.add, [p[kb] for kb in ks]), jnp.sum, 0.0)
            rl.append(1.0 / l)
            for kb in ks:
                pb = p[kb].astype(bf16)
                if kb == rb:
                    pi = pltpu.bitcast(pb, i32)
                    pp[kb + 8, rb] = pltpu.bitcast(pi & trip, bf16)
                    if not edge:
                        pp[kb, rb] = pltpu.bitcast(pi & (~trip), bf16)
                elif rb > kb:
                    pp[kb + 8, rb] = pb
                else:
                    pp[kb, rb] = pb
        return pp, rl

    def a_vload(g, blk, edge):
        r0 = pl.multiple_of(blk * R, R)
        k0 = 8 if edge else 0
        return v_s[g, pl.ds(r0 + 32 * k0, 32 * (16 - k0)), :]

    def a_values(g, blk, edge, vw, pp, rl):
        k0 = 8 if edge else 0
        acc = [None] * 8
        for kb in range(k0, 16):
            vbd = stack_heads(vw[32 * (kb - k0):32 * (kb - k0) + 32])
            rbs = list(range(0, kb + 1)) if kb < 8 else list(range(kb - 8, 8))
            p = jnp.concatenate([pp[kb, rb] for rb in rbs], axis=0)
            o = jnp.dot(p, vbd, preferred_element_type=f32)
            for n, rb in enumerate(rbs):
                ob = o[32 * n:32 * n + 32]
                acc[rb] = ob if acc[rb] is None else acc[rb] + ob
        for rb in range(8):
            o_s[blk % 2, g, 32 * rb:32 * rb + 32, :] = (acc[rb] * rl[rb]).astype(bf16)

    def b_scores(g, blk):
        r0 = pl.multiple_of(blk * R, R)
        q = q_s[g, pl.ds(r0, R), :]
        kw = k_s[g, pl.ds(r0 + (PAD - 32), R + 32), :]
        ss = {}
        for kb in range(-1, 8):
            kbd = stack_heads(kw[32 * (kb + 1):32 * (kb + 2)])
            qq = q[0:16] if kb < 0 else q[32 * kb:min(32 * kb + 48, R)]
            ss[kb] = lax.dot_general(qq, kbd, _NT, preferred_element_type=f32)
        return ss

    def b_softmax(ss, blk):
        tri = tri_mask(16)
        kk = lax.broadcasted_iota(i32, (32, 128), 1) % DH
        row = lax.broadcasted_iota(i32, (32, 128), 0)
        dl = (row - kk) & 31
        ok = (dl <= 14) & ((dl & 1) == 0)
        tiles = []
        for rb in range(8):
            prev = ss[-1] if rb == 0 else ss[rb - 1][32:48]
            top = jnp.where(tri, ss[rb][0:16], prev)
            tile = jnp.concatenate([top, ss[rb][16:32]], axis=0)
            okr = ok & ((kk <= row) | (blk > 0)) if rb == 0 else ok
            tiles.append(jnp.where(okr, tile, NEG))
        s = jnp.concatenate(tiles, axis=0)
        m = seg_reduce(s, jnp.max, -jnp.inf)
        p = jnp.exp2(s - m)
        rl = 1.0 / seg_reduce(p, jnp.sum, 0.0)
        pb = p.astype(bf16)
        trip = tri_mask_packed(16)
        own, prv = [], []
        for rb in range(8):
            pi = pltpu.bitcast(pb[32 * rb:32 * rb + 16], i32)
            own.append(jnp.concatenate(
                [pltpu.bitcast(pi & trip, bf16), pb[32 * rb + 16:32 * rb + 32]], axis=0))
            prv.append(pltpu.bitcast(pi & (~trip), bf16))
        return own, prv, rl

    def b_vload(g, blk):
        r0 = pl.multiple_of(blk * R, R)
        return v_s[g, pl.ds(r0 + (PAD - 32), R + 32), :]

    def b_values(g, blk, vw, own, prv, rl):
        outs = {}
        for kb in range(-1, 8):
            vbd = stack_heads(vw[32 * (kb + 1):32 * (kb + 2)])
            if kb < 0:
                p = prv[0]
            elif kb < 7:
                p = jnp.concatenate([own[kb], prv[kb + 1]], axis=0)
            else:
                p = own[kb]
            outs[kb] = jnp.dot(p, vbd, preferred_element_type=f32)
        for rb in range(8):
            prev = outs[-1] if rb == 0 else outs[rb - 1][32:48]
            o = jnp.concatenate([outs[rb][0:16] + prev, outs[rb][16:32]], axis=0)
            o_s[blk % 2, g, 32 * rb:32 * rb + 32, :] = (o * rl[32 * rb:32 * rb + 32]).astype(bf16)

    def out_dma(blk):
        r0 = pl.multiple_of(blk * R, R)
        return pltpu.make_async_copy(xio.at[pl.ds(r0, R), :], out_hbm.at[pl.ds(r0, R), :],
                                     sems.at[5])

    def run_steps(typ, pair, i_lo, i_hi, edge=False, tail=False):
        nc = NG // GU

        def body(t, c):
            i = i_lo + t // nc
            gs = [(t % nc) * GU + u for u in range(GU)]
            if typ == 0:
                ss = [a_scores(g, i, edge) for g in gs]
                vws = [a_vload(g, i, edge) for g in gs]
            else:
                ss = [b_scores(g, i) for g in gs]
                vws = [b_vload(g, i) for g in gs]
            if not tail:
                for g in gs:
                    part_ln((i + 2) % NB, g)
            if typ == 0:
                ps = [a_softmax(s_, edge) for s_ in ss]
            else:
                ps = [b_softmax(s_, i) for s_ in ss]

            final = pair == 1 and typ == 1
            if not (edge and pair == 0):
                for g in gs:
                    if i_lo >= 1:
                        part_out(typ, i - 1, g, final)
                    else:
                        part_out((typ + NB + (i - 1) // NB) % 2, (i + NB - 1) % NB, g, False)

            def qkvs(gl):
                if not tail:
                    for g in gl:
                        part_qkv((typ + (i + 1) // NB) % 2, (i + 1) % NB, g)

            qkvs(gs[:NQ1])
            for g, vw, p_ in zip(gs, vws, ps):
                if typ == 0:
                    a_values(g, i, edge, vw, *p_)
                else:
                    b_values(g, i, vw, *p_)
            qkvs(gs[NQ1:])
            if final and i_lo >= 1:
                @pl.when(t % nc == nc - 1)
                def _():
                    out_dma(i - 1).start()
            return c
        lax.fori_loop(0, (i_hi - i_lo) * nc, body, 0)

    cp_x0.wait()
    lax.fori_loop(0, 2, cvt, 0)

    def pro_ln(t, c):
        for r in range(NG):
            part_ln(t, r)
        return c
    lax.fori_loop(0, 2, pro_ln, 0)

    for g in range(NG):
        for cp in cp_wqa(g):
            cp.wait()
        if g + 2 < NG:
            for cp in cp_wqa(g + 2):
                cp.start()
        if g == NG - 3:
            cp_x1.start()
        if g == NG - 1:
            cp_woa.start()
            cp_wqb.start()
            cp_wob.start()
        part_qkv(0, 0, g)
    cp_x1.wait()
    lax.fori_loop(2, NB, cvt, 0)

    for pair in range(2):
        run_steps(0, pair, 0, 1, edge=True)
        if pair == 0:
            cp_woa.wait()
            cp_wqb.wait()
        run_steps(0, pair, 1, NB)
        if pair == 0:
            cp_wob.wait()
            run_steps(1, pair, 0, NB)
        else:
            run_steps(1, pair, 0, 1)
            run_steps(1, pair, 1, NB - 1)
            run_steps(1, pair, NB - 1, NB, tail=True)

    def epi(g, c):
        part_out(1, NB - 1, g, True)
        return c
    lax.fori_loop(0, NG, epi, 0)
    out_dma(NB - 1).start()
    pltpu.make_async_copy(xio, out_hbm, sems.at[5]).wait()


@jax.jit
def pallas_interleave_layers__sliding_block__sliding_local_dilated__prompt_kernel(
    A_x: jax.Array,
    A_wqkv: jax.Array,
    A_wo: jax.Array,
    B_x: jax.Array,
    B_wqkv: jax.Array,
    B_wo: jax.Array,
):
    del B_x
    bf16, f32 = jnp.bfloat16, jnp.float32
    any_spec = pl.BlockSpec(memory_space=pl.ANY)
    out = pl.pallas_call(
        _kernel,
        in_specs=[any_spec] * 5,
        out_specs=any_spec,
        out_shape=jax.ShapeDtypeStruct((S, D), bf16),
        scratch_shapes=[
            pltpu.VMEM((S, D), f32),
            pltpu.VMEM((S, D), bf16),
            pltpu.VMEM((2, D, 3 * D), bf16),
            pltpu.VMEM((2, D, D), bf16),
            pltpu.VMEM((NG, S, 128), bf16),
            pltpu.VMEM((NG, PAD + S, 128), bf16),
            pltpu.VMEM((NG, PAD + S, 128), bf16),
            pltpu.VMEM((2, NG, R, 128), bf16),
            pltpu.VMEM((2, R, D), bf16),
            pltpu.SemaphoreType.DMA((14,)),
        ],
        compiler_params=pltpu.CompilerParams(vmem_limit_bytes=100 * 1024 * 1024),
    )(A_x.reshape(S, D), A_wqkv, A_wo, B_wqkv, B_wo)
    return out.reshape(1, S, D)
```

```python
import functools
import math

import jax
import jax.numpy as jnp
from jax import lax
import jax.experimental.pallas as pl
import jax.experimental.pallas.tpu as pltpu

S = 2048
D = 1024
NG = 8
DH = 32
PAD = 256
R = 256
NB = S // R
QORDER = ((0,), (1, 2))
HD = D // 2
EPS = 1e-5
NEG = -1e9
QSCALE = (DH ** -0.5) * math.log2(math.e)

_NT = (((1,), (1,)), ((), ()))


def _strassen_lhs(x11, x12, x21, x22):
    return (x11 + x22, x21 + x22, x11, x22, x11 + x12, x21 - x11, x12 - x22)


def _kernel(x_hbm, wqa_hbm, woa_hbm, wqb_hbm, wob_hbm, out_hbm,
            xres, xio, wq, wo, ws, q_s, k_s, v_s, o_s, xn_s, sems):
    f32, bf16, i32 = jnp.float32, jnp.bfloat16, jnp.int32

    cp_x0 = pltpu.make_async_copy(x_hbm.at[0:2 * R], xio.at[0:2 * R], sems.at[0])
    cp_x1 = pltpu.make_async_copy(x_hbm.at[2 * R:S], xio.at[2 * R:S], sems.at[1])
    cp_woa = pltpu.make_async_copy(woa_hbm, wo.at[0], sems.at[2])
    cp_wqb = pltpu.make_async_copy(wqb_hbm, wq.at[1], sems.at[3])
    cp_wob = pltpu.make_async_copy(wob_hbm, wo.at[1], sems.at[4])

    def cp_wqa(u):
        c = (u % 3) * D + (u // 3) * 128
        return [pltpu.make_async_copy(wqa_hbm.at[:, pl.ds(c + h * HD, 128)],
                                      wq.at[0, :, pl.ds(c + h * HD, 128)],
                                      sems.at[6 + u]) for h in range(2)]

    cp_x0.start()
    for u in range(3):
        for cp in cp_wqa(u):
            cp.start()

    k_s[:, PAD - 32:PAD, :] = jnp.zeros((NG, 32, 128), bf16)
    v_s[:, PAD - 32:PAD, :] = jnp.zeros((NG, 32, 128), bf16)

    def cvt(i, c):
        r0 = pl.multiple_of(i * R, R)
        xres[pl.ds(r0, R), :] = xio[pl.ds(r0, R), :].astype(f32)
        return c

    def lane_group(n):
        return lax.broadcasted_iota(i32, (n, 128), 1) // DH

    def stack_heads(q):
        n = q.shape[0]
        qi = pltpu.bitcast(q, i32)
        lg = lane_group(n // 2)
        parts = [pltpu.bitcast(jnp.where(lg == h, qi, 0), bf16) for h in range(4)]
        return jnp.concatenate(parts, axis=0)

    def prep_weights(raw, c0, dst):
        def ld(r, c):
            return raw[r * HD:(r + 1) * HD, pl.ds(pl.multiple_of(c0 + c * HD, 128), 128)]
        b11, b12, b21, b22 = ld(0, 0), ld(0, 1), ld(1, 0), ld(1, 1)
        w11, w12, w21, w22 = (b.astype(f32) for b in (b11, b12, b21, b22))
        dst[0] = (w11 + w22).astype(bf16)
        dst[1] = b11
        dst[2] = (w12 - w22).astype(bf16)
        dst[3] = (w21 - w11).astype(bf16)
        dst[4] = b22
        dst[5] = (w11 + w12).astype(bf16)
        dst[6] = (w21 + w22).astype(bf16)

    def prep_qkv(wi, which, pi_):
        prep_weights(wq.at[wi], which * D + pi_ * 128, ws.at[wi, which * 4 + pi_])

    def prep_out(wi, pi_):
        prep_weights(wo.at[wi], pi_ * 128, ws.at[wi, 12 + pi_])

    def strassen(lhs, rhs):
        def mm(i):
            return jnp.dot(lhs[i], rhs[i], preferred_element_type=f32)
        m1 = mm(0)
        m2 = mm(1)
        c22 = m1 - m2
        m4 = mm(3)
        c21 = m2 + m4
        c11 = m1 + m4
        m3 = mm(2)
        c22 = c22 + m3
        m5 = mm(4)
        c12 = m3 + m5
        c11 = c11 - m5
        c22 = c22 + mm(5)
        c11 = c11 + mm(6)
        return c11, c12, c21, c22

    def part_ln(blk, r):
        r16 = pl.multiple_of(r * 16, 16)

        def ln(off):
            x = xres[pl.ds(pl.multiple_of(blk * R + off + r16, 16), 16), :]
            m = jnp.mean(x, axis=-1, keepdims=True)
            xc = x - m
            v = jnp.mean(xc * xc, axis=-1, keepdims=True)
            return xc * lax.rsqrt(v + EPS)
        top, bot = ln(0), ln(R // 2)
        for i, l in enumerate(_strassen_lhs(top[:, :HD], top[:, HD:], bot[:, :HD], bot[:, HD:])):
            xn_s[blk % 2, i, pl.ds(r16, 16), :] = l.astype(bf16)

    def part_qkv(wi, blk, pi_, whichs=(0, 1, 2)):
        r0 = pl.multiple_of(blk * R, R)
        for which in whichs:
            cs = strassen(xn_s.at[blk % 2], ws.at[wi, which * 4 + pi_])
            for n, c in enumerate(cs):
                g = pi_ + 4 * (n % 2)
                rr = r0 + (n // 2) * (R // 2)
                if which == 0:
                    q_s[g, pl.ds(rr, R // 2), :] = (c * QSCALE).astype(bf16)
                elif which == 1:
                    k_s[g, pl.ds(rr + PAD, R // 2), :] = c.astype(bf16)
                else:
                    v_s[g, pl.ds(rr + PAD, R // 2), :] = c.astype(bf16)

    def part_out(wi, blk, pi_, last):
        r0 = pl.multiple_of(blk * R, R)
        cs = strassen(o_s.at[blk % 2], ws.at[wi, 12 + pi_])
        for n, c in enumerate(cs):
            c0 = pl.multiple_of(pi_ * 128 + HD * (n % 2), 128)
            rr = r0 + (n // 2) * (R // 2)
            y = c + xres[pl.ds(rr, R // 2), pl.ds(c0, 128)]
            if last:
                xio[pl.ds(rr, R // 2), pl.ds(c0, 128)] = y.astype(bf16)
            else:
                xres[pl.ds(rr, R // 2), pl.ds(c0, 128)] = y

    def store_o(blk, pi_, oa, ob):
        c0 = pl.multiple_of(pi_ * 128, 128)
        h = R // 2
        for i, l in enumerate(_strassen_lhs(oa[:h], ob[:h], oa[h:], ob[h:])):
            o_s[blk % 2, i, :, pl.ds(c0, 128)] = l.astype(bf16)

    def seg_reduce(x, op, fill):
        lg = lane_group(x.shape[0])
        r = None
        for h in range(4):
            rh = op(jnp.where(lg == h, x, fill), axis=-1, keepdims=True)
            r = jnp.broadcast_to(rh, x.shape) if r is None else jnp.where(lg == h, rh, r)
        return r

    def tri_mask(n):
        kk = lax.broadcasted_iota(i32, (n, 128), 1) % DH
        return kk <= lax.broadcasted_iota(i32, (n, 128), 0)

    def tri_mask_packed(n):
        kk = lax.broadcasted_iota(i32, (n // 2, 128), 1) % DH
        row2 = lax.broadcasted_iota(i32, (n // 2, 128), 0) * 2
        return jnp.where(kk <= row2, 0x0000FFFF, 0) | jnp.where(kk <= row2 + 1, -65536, 0)

    def a_scores(g, blk, edge):
        r0 = pl.multiple_of(blk * R, R)
        q = q_s[g, pl.ds(r0, R), :]
        k0 = 8 if edge else 0
        kw = k_s[g, pl.ds(r0 + 32 * k0, 32 * (16 - k0)), :]
        ss = {}
        for kb in range(k0, 16):
            kbd = stack_heads(kw[32 * (kb - k0):32 * (kb - k0) + 32])
            qq = q[0:32 * kb + 32] if kb < 8 else q[32 * (kb - 8):R]
            ss[kb] = lax.dot_general(qq, kbd, _NT, preferred_element_type=f32)
        return ss

    def a_softmax(ss, edge):
        tri = tri_mask(32)
        t = {}
        for kb in range(8):
            for rb in range(8):
                if rb == kb:
                    old = NEG if edge else ss[kb][32 * kb:32 * kb + 32]
                    t[kb, rb] = jnp.where(tri, ss[kb + 8][0:32], old)
                elif rb > kb:
                    t[kb, rb] = ss[kb + 8][32 * (rb - kb):32 * (rb - kb) + 32]
                elif not edge:
                    t[kb, rb] = ss[kb][32 * rb:32 * rb + 32]
        trip = tri_mask_packed(32)
        pp, rl = {}, []
        for rb in range(8):
            ks = [kb for kb in range(8) if (kb, rb) in t]
            m = functools.reduce(jnp.maximum, [t[kb, rb] for kb in ks])
            m = seg_reduce(m, jnp.max, -jnp.inf)
            p = {kb: jnp.exp2(t[kb, rb] - m) for kb in ks}
            l = seg_reduce(functools.reduce(jnp.add, [p[kb] for kb in ks]), jnp.sum, 0.0)
            rl.append(1.0 / l)
            for kb in ks:
                pb = p[kb].astype(bf16)
                if kb == rb:
                    pi = pltpu.bitcast(pb, i32)
                    pp[kb + 8, rb] = pltpu.bitcast(pi & trip, bf16)
                    if not edge:
                        pp[kb, rb] = pltpu.bitcast(pi & (~trip), bf16)
                elif rb > kb:
                    pp[kb + 8, rb] = pb
                else:
                    pp[kb, rb] = pb
        return pp, rl

    def a_vload(g, blk, edge):
        r0 = pl.multiple_of(blk * R, R)
        k0 = 8 if edge else 0
        return v_s[g, pl.ds(r0 + 32 * k0, 32 * (16 - k0)), :]

    def a_values(edge, vw, pp, rl):
        k0 = 8 if edge else 0
        acc = [None] * 8
        for kb in range(k0, 16):
            vbd = stack_heads(vw[32 * (kb - k0):32 * (kb - k0) + 32])
            rbs = list(range(0, kb + 1)) if kb < 8 else list(range(kb - 8, 8))
            p = jnp.concatenate([pp[kb, rb] for rb in rbs], axis=0)
            o = jnp.dot(p, vbd, preferred_element_type=f32)
            for n, rb in enumerate(rbs):
                ob = o[32 * n:32 * n + 32]
                acc[rb] = ob if acc[rb] is None else acc[rb] + ob
        return jnp.concatenate([acc[rb] * rl[rb] for rb in range(8)], axis=0)

    def b_scores(g, blk):
        r0 = pl.multiple_of(blk * R, R)
        q = q_s[g, pl.ds(r0, R), :]
        kw = k_s[g, pl.ds(r0 + (PAD - 32), R + 32), :]
        ss = {}
        for kb in range(-1, 8):
            kbd = stack_heads(kw[32 * (kb + 1):32 * (kb + 2)])
            qq = q[0:16] if kb < 0 else q[32 * kb:min(32 * kb + 48, R)]
            ss[kb] = lax.dot_general(qq, kbd, _NT, preferred_element_type=f32)
        return ss

    def b_softmax(ss, blk):
        tri = tri_mask(16)
        kk = lax.broadcasted_iota(i32, (32, 128), 1) % DH
        row = lax.broadcasted_iota(i32, (32, 128), 0)
        dl = (row - kk) & 31
        ok = (dl <= 14) & ((dl & 1) == 0)
        tiles = []
        for rb in range(8):
            prev = ss[-1] if rb == 0 else ss[rb - 1][32:48]
            top = jnp.where(tri, ss[rb][0:16], prev)
            tile = jnp.concatenate([top, ss[rb][16:32]], axis=0)
            okr = ok & ((kk <= row) | (blk > 0)) if rb == 0 else ok
            tiles.append(jnp.where(okr, tile, NEG))
        s = jnp.concatenate(tiles, axis=0)
        m = seg_reduce(s, jnp.max, -jnp.inf)
        p = jnp.exp2(s - m)
        rl = 1.0 / seg_reduce(p, jnp.sum, 0.0)
        pb = p.astype(bf16)
        trip = tri_mask_packed(16)
        own, prv = [], []
        for rb in range(8):
            pi = pltpu.bitcast(pb[32 * rb:32 * rb + 16], i32)
            own.append(jnp.concatenate(
                [pltpu.bitcast(pi & trip, bf16), pb[32 * rb + 16:32 * rb + 32]], axis=0))
            prv.append(pltpu.bitcast(pi & (~trip), bf16))
        return own, prv, rl

    def b_vload(g, blk):
        r0 = pl.multiple_of(blk * R, R)
        return v_s[g, pl.ds(r0 + (PAD - 32), R + 32), :]

    def b_values(vw, own, prv, rl):
        outs = {}
        for kb in range(-1, 8):
            vbd = stack_heads(vw[32 * (kb + 1):32 * (kb + 2)])
            if kb < 0:
                p = prv[0]
            elif kb < 7:
                p = jnp.concatenate([own[kb], prv[kb + 1]], axis=0)
            else:
                p = own[kb]
            outs[kb] = jnp.dot(p, vbd, preferred_element_type=f32)
        res = []
        for rb in range(8):
            prev = outs[-1] if rb == 0 else outs[rb - 1][32:48]
            o = jnp.concatenate([outs[rb][0:16] + prev, outs[rb][16:32]], axis=0)
            res.append(o)
        return jnp.concatenate(res, axis=0) * rl

    def out_dma(blk):
        r0 = pl.multiple_of(blk * R, R)
        return pltpu.make_async_copy(xio.at[pl.ds(r0, R), :], out_hbm.at[pl.ds(r0, R), :],
                                     sems.at[5])

    def run_steps(typ, pair, i_lo, i_hi, edge=False, tail=False):
        nc = NG // 2

        def body(t, c):
            i = i_lo + t // nc
            pi_ = t % nc
            gs = [pi_, pi_ + 4]
            if typ == 0:
                ss = [a_scores(g, i, edge) for g in gs]
                vws = [a_vload(g, i, edge) for g in gs]
            else:
                ss = [b_scores(g, i) for g in gs]
                vws = [b_vload(g, i) for g in gs]
            if not tail:
                for u in range(2):
                    part_ln((i + 2) % NB, 2 * pi_ + u)
            if typ == 0:
                ps = [a_softmax(s_, edge) for s_ in ss]
            else:
                ps = [b_softmax(s_, i) for s_ in ss]
            final = pair == 1 and typ == 1
            if not (edge and pair == 0):
                if i_lo >= 1:
                    part_out(typ, i - 1, pi_, final)
                else:
                    part_out((typ + NB + (i - 1) // NB) % 2, (i + NB - 1) % NB, pi_, False)

            def qkvs(whichs):
                if not tail:
                    part_qkv((typ + (i + 1) // NB) % 2, (i + 1) % NB, pi_, whichs)

            qkvs(QORDER[0])
            if typ == 0:
                os_ = [a_values(edge, vw, *p_) for vw, p_ in zip(vws, ps)]
            else:
                os_ = [b_values(vw, *p_) for vw, p_ in zip(vws, ps)]
            store_o(i, pi_, *os_)
            qkvs(QORDER[1])
            if final and i_lo >= 1:
                @pl.when(pi_ == nc - 1)
                def _():
                    out_dma(i - 1).start()
            return c
        lax.fori_loop(0, (i_hi - i_lo) * nc, body, 0)

    cp_x0.wait()
    lax.fori_loop(0, 2, cvt, 0)

    def pro_ln(t, c):
        for r in range(NG):
            part_ln(t, r)
        return c
    lax.fori_loop(0, 2, pro_ln, 0)

    for u in range(12):
        for cp in cp_wqa(u):
            cp.wait()
        if u + 3 < 12:
            for cp in cp_wqa(u + 3):
                cp.start()
        if u == 7:
            cp_x1.start()
        if u == 10:
            cp_woa.start()
        if u == 11:
            cp_wqb.start()
            cp_wob.start()
        prep_qkv(0, u % 3, u // 3)
        part_qkv(0, 0, u // 3, (u % 3,))
    cp_x1.wait()
    lax.fori_loop(2, NB, cvt, 0)

    def prep_loop(fn, n):
        def body(t, c):
            fn(t)
            return c
        lax.fori_loop(0, n, body, 0)

    for pair in range(2):
        run_steps(0, pair, 0, 1, edge=True)
        if pair == 0:
            cp_woa.wait()
            prep_loop(lambda t: prep_out(0, t), 4)
            run_steps(0, pair, 1, 4)
            cp_wqb.wait()
            cp_wob.wait()
            for which in range(3):
                prep_loop(lambda t: prep_qkv(1, which, t), 4)
            prep_loop(lambda t: prep_out(1, t), 4)
            run_steps(0, pair, 4, NB)
            run_steps(1, pair, 0, NB)
        else:
            run_steps(0, pair, 1, NB)
            run_steps(1, pair, 0, 1)
            run_steps(1, pair, 1, NB - 1)
            run_steps(1, pair, NB - 1, NB, tail=True)

    def epi(t, c):
        part_out(1, NB - 1, t, True)
        return c
    lax.fori_loop(0, 4, epi, 0)
    out_dma(NB - 1).start()
    pltpu.make_async_copy(xio, out_hbm, sems.at[5]).wait()


@jax.jit
def pallas_interleave_layers__sliding_block__sliding_local_dilated__prompt_kernel(
    A_x: jax.Array,
    A_wqkv: jax.Array,
    A_wo: jax.Array,
    B_x: jax.Array,
    B_wqkv: jax.Array,
    B_wo: jax.Array,
):
    del B_x
    bf16, f32 = jnp.bfloat16, jnp.float32
    any_spec = pl.BlockSpec(memory_space=pl.ANY)
    out = pl.pallas_call(
        _kernel,
        in_specs=[any_spec] * 5,
        out_specs=any_spec,
        out_shape=jax.ShapeDtypeStruct((S, D), bf16),
        scratch_shapes=[
            pltpu.VMEM((S, D), f32),
            pltpu.VMEM((S, D), bf16),
            pltpu.VMEM((2, D, 3 * D), bf16),
            pltpu.VMEM((2, D, D), bf16),
            pltpu.VMEM((2, 16, 7, HD, 128), bf16),
            pltpu.VMEM((NG, S, 128), bf16),
            pltpu.VMEM((NG, PAD + S, 128), bf16),
            pltpu.VMEM((NG, PAD + S, 128), bf16),
            pltpu.VMEM((2, 7, R // 2, HD), bf16),
            pltpu.VMEM((2, 7, R // 2, HD), bf16),
            pltpu.SemaphoreType.DMA((18,)),
        ],
        compiler_params=pltpu.CompilerParams(vmem_limit_bytes=100 * 1024 * 1024),
    )(A_x.reshape(S, D), A_wqkv, A_wo, B_wqkv, B_wo)
    return out.reshape(1, S, D)
```

```python
import functools
import math

import jax
import jax.numpy as jnp
from jax import lax
import jax.experimental.pallas as pl
import jax.experimental.pallas.tpu as pltpu

S = 2048
D = 1024
NG = 8
DH = 32
PAD = 256
R = 256
NB = S // R
ORDER = ("s0 l o s1 p0 v0 p1 v1 p2".split(), "s0 s1 l o p0 v0 v1 p1 p2".split())
HD = D // 2
EPS = 1e-5
NEG = -1e9
QSCALE = (DH ** -0.5) * math.log2(math.e)

_NT = (((1,), (1,)), ((), ()))


def _strassen_lhs(x11, x12, x21, x22):
    return (x11 + x22, x21 + x22, x11, x22, x11 + x12, x21 - x11, x12 - x22)


def _kernel(x_hbm, wqa_hbm, woa_hbm, wqb_hbm, wob_hbm, out_hbm,
            xres, xio, wq, wo, ws, q_s, k_s, v_s, o_s, xn_s, sems):
    f32, bf16, i32 = jnp.float32, jnp.bfloat16, jnp.int32

    cp_x0 = pltpu.make_async_copy(x_hbm.at[0:2 * R], xio.at[0:2 * R], sems.at[0])
    cp_x1 = pltpu.make_async_copy(x_hbm.at[2 * R:S], xio.at[2 * R:S], sems.at[1])
    cp_woa = pltpu.make_async_copy(woa_hbm, wo.at[0], sems.at[2])
    cp_wqb = pltpu.make_async_copy(wqb_hbm, wq.at[1], sems.at[3])
    cp_wob = pltpu.make_async_copy(wob_hbm, wo.at[1], sems.at[4])

    def cp_wqa(u):
        c = (u % 3) * D + (u // 3) * 128
        return [pltpu.make_async_copy(wqa_hbm.at[:, pl.ds(c + h * HD, 128)],
                                      wq.at[0, :, pl.ds(c + h * HD, 128)],
                                      sems.at[6 + u]) for h in range(2)]

    cp_x0.start()
    for u in range(3):
        for cp in cp_wqa(u):
            cp.start()

    k_s[:, PAD - 32:PAD, :] = jnp.zeros((NG, 32, 128), bf16)
    v_s[:, PAD - 32:PAD, :] = jnp.zeros((NG, 32, 128), bf16)

    def cvt(i, c):
        r0 = pl.multiple_of(i * R, R)
        xres[pl.ds(r0, R), :] = xio[pl.ds(r0, R), :].astype(f32)
        return c

    def lane_group(n):
        return lax.broadcasted_iota(i32, (n, 128), 1) // DH

    def stack_heads(q):
        n = q.shape[0]
        qi = pltpu.bitcast(q, i32)
        lg = lane_group(n // 2)
        parts = [pltpu.bitcast(jnp.where(lg == h, qi, 0), bf16) for h in range(4)]
        return jnp.concatenate(parts, axis=0)

    def prep_weights(raw, c0, dst):
        ch = 64
        for r0 in range(0, HD, ch):
            def ld(r, c):
                return raw[r * HD + r0:r * HD + r0 + ch,
                           pl.ds(pl.multiple_of(c0 + c * HD, 128), 128)]
            b11, b12, b21, b22 = ld(0, 0), ld(0, 1), ld(1, 0), ld(1, 1)
            w11, w12, w21, w22 = (b.astype(f32) for b in (b11, b12, b21, b22))
            rows = slice(r0, r0 + ch)
            dst[0, rows] = (w11 + w22).astype(bf16)
            dst[1, rows] = b11
            dst[2, rows] = (w12 - w22).astype(bf16)
            dst[3, rows] = (w21 - w11).astype(bf16)
            dst[4, rows] = b22
            dst[5, rows] = (w11 + w12).astype(bf16)
            dst[6, rows] = (w21 + w22).astype(bf16)

    def prep_qkv(wi, which, pi_):
        prep_weights(wq.at[wi], which * D + pi_ * 128, ws.at[wi, which * 4 + pi_])

    def prep_out(wi, pi_):
        prep_weights(wo.at[wi], pi_ * 128, ws.at[wi, 12 + pi_])

    def strassen(lhs, rhs):
        def mm(i):
            return jnp.dot(lhs[i], rhs[i], preferred_element_type=f32)
        m1 = mm(0)
        m2 = mm(1)
        c22 = m1 - m2
        m4 = mm(3)
        c21 = m2 + m4
        c11 = m1 + m4
        m3 = mm(2)
        c22 = c22 + m3
        m5 = mm(4)
        c12 = m3 + m5
        c11 = c11 - m5
        c22 = c22 + mm(5)
        c11 = c11 + mm(6)
        return c11, c12, c21, c22

    def part_ln(blk, r):
        r16 = pl.multiple_of(r * 16, 16)

        def ln(off):
            x = xres[pl.ds(pl.multiple_of(blk * R + off + r16, 16), 16), :]
            m = jnp.mean(x, axis=-1, keepdims=True)
            xc = x - m
            v = jnp.mean(xc * xc, axis=-1, keepdims=True)
            return xc * lax.rsqrt(v + EPS)
        top, bot = ln(0), ln(R // 2)
        for i, l in enumerate(_strassen_lhs(top[:, :HD], top[:, HD:], bot[:, :HD], bot[:, HD:])):
            xn_s[blk % 2, i, pl.ds(r16, 16), :] = l.astype(bf16)

    def part_qkv(wi, blk, pi_, whichs=(0, 1, 2)):
        r0 = pl.multiple_of(blk * R, R)
        for which in whichs:
            cs = strassen(xn_s.at[blk % 2], ws.at[wi, which * 4 + pi_])
            for n, c in enumerate(cs):
                g = pi_ + 4 * (n % 2)
                rr = r0 + (n // 2) * (R // 2)
                if which == 0:
                    q_s[g, pl.ds(rr, R // 2), :] = (c * QSCALE).astype(bf16)
                elif which == 1:
                    k_s[g, pl.ds(rr + PAD, R // 2), :] = c.astype(bf16)
                else:
                    v_s[g, pl.ds(rr + PAD, R // 2), :] = c.astype(bf16)

    def part_out(wi, blk, pi_, last):
        r0 = pl.multiple_of(blk * R, R)
        cs = strassen(o_s.at[blk % 2], ws.at[wi, 12 + pi_])
        for n, c in enumerate(cs):
            c0 = pl.multiple_of(pi_ * 128 + HD * (n % 2), 128)
            rr = r0 + (n // 2) * (R // 2)
            y = c + xres[pl.ds(rr, R // 2), pl.ds(c0, 128)]
            if last:
                xio[pl.ds(rr, R // 2), pl.ds(c0, 128)] = y.astype(bf16)
            else:
                xres[pl.ds(rr, R // 2), pl.ds(c0, 128)] = y

    def store_o(blk, pi_, oa, ob):
        c0 = pl.multiple_of(pi_ * 128, 128)
        h = R // 2
        for i, l in enumerate(_strassen_lhs(oa[:h], ob[:h], oa[h:], ob[h:])):
            o_s[blk % 2, i, :, pl.ds(c0, 128)] = l.astype(bf16)

    def seg_reduce(x, op, fill):
        lg = lane_group(x.shape[0])
        r = None
        for h in range(4):
            rh = op(jnp.where(lg == h, x, fill), axis=-1, keepdims=True)
            r = jnp.broadcast_to(rh, x.shape) if r is None else jnp.where(lg == h, rh, r)
        return r

    def tri_mask(n):
        kk = lax.broadcasted_iota(i32, (n, 128), 1) % DH
        return kk <= lax.broadcasted_iota(i32, (n, 128), 0)

    def tri_mask_packed(n):
        kk = lax.broadcasted_iota(i32, (n // 2, 128), 1) % DH
        row2 = lax.broadcasted_iota(i32, (n // 2, 128), 0) * 2
        return jnp.where(kk <= row2, 0x0000FFFF, 0) | jnp.where(kk <= row2 + 1, -65536, 0)

    def a_load(g, blk, edge):
        r0 = pl.multiple_of(blk * R, R)
        k0 = 8 if edge else 0
        w = pl.ds(r0 + 32 * k0, 32 * (16 - k0))
        return q_s[g, pl.ds(r0, R), :], k_s[g, w, :], v_s[g, w, :]

    def a_scores(q, kw, edge):
        k0 = 8 if edge else 0
        ss = {}
        for kb in range(k0, 16):
            kbd = stack_heads(kw[32 * (kb - k0):32 * (kb - k0) + 32])
            qq = q[0:32 * kb + 32] if kb < 8 else q[32 * (kb - 8):R]
            ss[kb] = lax.dot_general(qq, kbd, _NT, preferred_element_type=f32)
        return ss

    def a_softmax(ss, edge):
        tri = tri_mask(32)
        t = {}
        for kb in range(8):
            for rb in range(8):
                if rb == kb:
                    old = NEG if edge else ss[kb][32 * kb:32 * kb + 32]
                    t[kb, rb] = jnp.where(tri, ss[kb + 8][0:32], old)
                elif rb > kb:
                    t[kb, rb] = ss[kb + 8][32 * (rb - kb):32 * (rb - kb) + 32]
                elif not edge:
                    t[kb, rb] = ss[kb][32 * rb:32 * rb + 32]
        trip = tri_mask_packed(32)
        pp, rl = {}, []
        for rb in range(8):
            ks = [kb for kb in range(8) if (kb, rb) in t]
            m = functools.reduce(jnp.maximum, [t[kb, rb] for kb in ks])
            m = seg_reduce(m, jnp.max, -jnp.inf)
            p = {kb: jnp.exp2(t[kb, rb] - m) for kb in ks}
            l = seg_reduce(functools.reduce(jnp.add, [p[kb] for kb in ks]), jnp.sum, 0.0)
            rl.append(1.0 / l)
            for kb in ks:
                pb = p[kb].astype(bf16)
                if kb == rb:
                    pi = pltpu.bitcast(pb, i32)
                    pp[kb + 8, rb] = pltpu.bitcast(pi & trip, bf16)
                    if not edge:
                        pp[kb, rb] = pltpu.bitcast(pi & (~trip), bf16)
                elif rb > kb:
                    pp[kb + 8, rb] = pb
                else:
                    pp[kb, rb] = pb
        return pp, rl

    def a_values(edge, vw, pp, rl):
        k0 = 8 if edge else 0
        acc = [None] * 8
        for kb in range(k0, 16):
            vbd = stack_heads(vw[32 * (kb - k0):32 * (kb - k0) + 32])
            rbs = list(range(0, kb + 1)) if kb < 8 else list(range(kb - 8, 8))
            p = jnp.concatenate([pp[kb, rb] for rb in rbs], axis=0)
            o = jnp.dot(p, vbd, preferred_element_type=f32)
            for n, rb in enumerate(rbs):
                ob = o[32 * n:32 * n + 32]
                acc[rb] = ob if acc[rb] is None else acc[rb] + ob
        return jnp.concatenate([acc[rb] * rl[rb] for rb in range(8)], axis=0)

    def b_load(g, blk):
        r0 = pl.multiple_of(blk * R, R)
        w = pl.ds(r0 + (PAD - 32), R + 32)
        return q_s[g, pl.ds(r0, R), :], k_s[g, w, :], v_s[g, w, :]

    def b_scores(q, kw):
        ss = {}
        for kb in range(-1, 8):
            kbd = stack_heads(kw[32 * (kb + 1):32 * (kb + 2)])
            qq = q[0:16] if kb < 0 else q[32 * kb:min(32 * kb + 48, R)]
            ss[kb] = lax.dot_general(qq, kbd, _NT, preferred_element_type=f32)
        return ss

    def b_softmax(ss, blk):
        tri = tri_mask(16)
        kk = lax.broadcasted_iota(i32, (32, 128), 1) % DH
        row = lax.broadcasted_iota(i32, (32, 128), 0)
        dl = (row - kk) & 31
        ok = (dl <= 14) & ((dl & 1) == 0)
        tiles = []
        for rb in range(8):
            prev = ss[-1] if rb == 0 else ss[rb - 1][32:48]
            top = jnp.where(tri, ss[rb][0:16], prev)
            tile = jnp.concatenate([top, ss[rb][16:32]], axis=0)
            okr = ok & ((kk <= row) | (blk > 0)) if rb == 0 else ok
            tiles.append(jnp.where(okr, tile, NEG))
        s = jnp.concatenate(tiles, axis=0)
        m = seg_reduce(s, jnp.max, -jnp.inf)
        p = jnp.exp2(s - m)
        rl = 1.0 / seg_reduce(p, jnp.sum, 0.0)
        pb = p.astype(bf16)
        trip = tri_mask_packed(16)
        own, prv = [], []
        for rb in range(8):
            pi = pltpu.bitcast(pb[32 * rb:32 * rb + 16], i32)
            own.append(jnp.concatenate(
                [pltpu.bitcast(pi & trip, bf16), pb[32 * rb + 16:32 * rb + 32]], axis=0))
            prv.append(pltpu.bitcast(pi & (~trip), bf16))
        return own, prv, rl

    def b_values(vw, own, prv, rl):
        outs = {}
        for kb in range(-1, 8):
            vbd = stack_heads(vw[32 * (kb + 1):32 * (kb + 2)])
            if kb < 0:
                p = prv[0]
            elif kb < 7:
                p = jnp.concatenate([own[kb], prv[kb + 1]], axis=0)
            else:
                p = own[kb]
            outs[kb] = jnp.dot(p, vbd, preferred_element_type=f32)
        res = []
        for rb in range(8):
            prev = outs[-1] if rb == 0 else outs[rb - 1][32:48]
            o = jnp.concatenate([outs[rb][0:16] + prev, outs[rb][16:32]], axis=0)
            res.append(o)
        return jnp.concatenate(res, axis=0) * rl

    def out_dma(blk):
        r0 = pl.multiple_of(blk * R, R)
        return pltpu.make_async_copy(xio.at[pl.ds(r0, R), :], out_hbm.at[pl.ds(r0, R), :],
                                     sems.at[5])

    def run_steps(typ, pair, i_lo, i_hi, edge=False, tail=False):
        nc = NG // 2

        def body(t, c):
            i = i_lo + t // nc
            pi_ = t % nc
            gs = [pi_, pi_ + 4]
            qkv = [a_load(g, i, edge) if typ == 0 else b_load(g, i) for g in gs]
            final = pair == 1 and typ == 1
            ps, os_ = {}, {}

            def score(n):
                q, kw, _ = qkv[n]
                if typ == 0:
                    ps[n] = a_softmax(a_scores(q, kw, edge), edge)
                else:
                    ps[n] = b_softmax(b_scores(q, kw), i)

            def value(n):
                if typ == 0:
                    os_[n] = a_values(edge, qkv[n][2], *ps[n])
                else:
                    os_[n] = b_values(qkv[n][2], *ps[n])
                if len(os_) == 2:
                    store_o(i, pi_, os_[0], os_[1])

            def out():
                if edge and pair == 0:
                    return
                if i_lo >= 1:
                    part_out(typ, i - 1, pi_, final)
                else:
                    part_out((typ + NB + (i - 1) // NB) % 2, (i + NB - 1) % NB, pi_, False)

            def ln():
                if not tail:
                    for u in range(2):
                        part_ln((i + 2) % NB, 2 * pi_ + u)

            for op in ORDER[typ]:
                if op[0] == "s":
                    score(int(op[1]))
                elif op[0] == "v":
                    value(int(op[1]))
                elif op[0] == "o":
                    out()
                elif op[0] == "l":
                    ln()
                elif not tail:
                    part_qkv((typ + (i + 1) // NB) % 2, (i + 1) % NB, pi_, (int(op[1]),))
            if final and i_lo >= 1:
                @pl.when(pi_ == nc - 1)
                def _():
                    out_dma(i - 1).start()
            return c
        lax.fori_loop(0, (i_hi - i_lo) * nc, body, 0)

    cp_x0.wait()
    lax.fori_loop(0, 2, cvt, 0)

    def pro_ln(t, c):
        for r in range(NG):
            part_ln(t, r)
        return c
    lax.fori_loop(0, 2, pro_ln, 0)

    for u in range(12):
        for cp in cp_wqa(u):
            cp.wait()
        if u + 3 < 12:
            for cp in cp_wqa(u + 3):
                cp.start()
        if u == 7:
            cp_x1.start()
        if u == 10:
            cp_woa.start()
        if u == 11:
            cp_wqb.start()
            cp_wob.start()
        prep_qkv(0, u % 3, u // 3)
        part_qkv(0, 0, u // 3, (u % 3,))
    cp_x1.wait()
    lax.fori_loop(2, NB, cvt, 0)

    def prep_loop(fn, n):
        def body(t, c):
            fn(t)
            return c
        lax.fori_loop(0, n, body, 0)

    for pair in range(2):
        run_steps(0, pair, 0, 1, edge=True)
        if pair == 0:
            cp_woa.wait()
            prep_loop(lambda t: prep_out(0, t), 4)
            run_steps(0, pair, 1, 4)
            cp_wqb.wait()
            cp_wob.wait()
            for which in range(3):
                prep_loop(lambda t: prep_qkv(1, which, t), 4)
            prep_loop(lambda t: prep_out(1, t), 4)
            run_steps(0, pair, 4, NB)
            run_steps(1, pair, 0, NB)
        else:
            run_steps(0, pair, 1, NB)
            run_steps(1, pair, 0, 1)
            run_steps(1, pair, 1, NB - 1)
            run_steps(1, pair, NB - 1, NB, tail=True)

    def epi(t, c):
        part_out(1, NB - 1, t, True)
        return c
    lax.fori_loop(0, 4, epi, 0)
    out_dma(NB - 1).start()
    pltpu.make_async_copy(xio, out_hbm, sems.at[5]).wait()


@jax.jit
def pallas_interleave_layers__sliding_block__sliding_local_dilated__prompt_kernel(
    A_x: jax.Array,
    A_wqkv: jax.Array,
    A_wo: jax.Array,
    B_x: jax.Array,
    B_wqkv: jax.Array,
    B_wo: jax.Array,
):
    del B_x
    bf16, f32 = jnp.bfloat16, jnp.float32
    any_spec = pl.BlockSpec(memory_space=pl.ANY)
    out = pl.pallas_call(
        _kernel,
        in_specs=[any_spec] * 5,
        out_specs=any_spec,
        out_shape=jax.ShapeDtypeStruct((S, D), bf16),
        scratch_shapes=[
            pltpu.VMEM((S, D), f32),
            pltpu.VMEM((S, D), bf16),
            pltpu.VMEM((2, D, 3 * D), bf16),
            pltpu.VMEM((2, D, D), bf16),
            pltpu.VMEM((2, 16, 7, HD, 128), bf16),
            pltpu.VMEM((NG, S, 128), bf16),
            pltpu.VMEM((NG, PAD + S, 128), bf16),
            pltpu.VMEM((NG, PAD + S, 128), bf16),
            pltpu.VMEM((2, 7, R // 2, HD), bf16),
            pltpu.VMEM((2, 7, R // 2, HD), bf16),
            pltpu.SemaphoreType.DMA((18,)),
        ],
        compiler_params=pltpu.CompilerParams(vmem_limit_bytes=100 * 1024 * 1024),
    )(A_x.reshape(S, D), A_wqkv, A_wo, B_wqkv, B_wo)
    return out.reshape(1, S, D)
```

```python
import functools
import math

import jax
import jax.numpy as jnp
from jax import lax
import jax.experimental.pallas as pl
import jax.experimental.pallas.tpu as pltpu

S = 2048
D = 1024
NG = 8
DH = 32
PAD = 256
R = 256
NB = S // R
ORDER = ("s0 l o s1 p0 p1 v0 v1 p2".split(), "s0 l o s1 p0 p1 v0 p2 v1".split())
HD = D // 2
EPS = 1e-5
NEG = -1e9
QSCALE = (DH ** -0.5) * math.log2(math.e)

_NT = (((1,), (1,)), ((), ()))


def _strassen_lhs(x11, x12, x21, x22):
    return (x11 + x22, x21 + x22, x11, x22, x11 + x12, x21 - x11, x12 - x22)


def _kernel(x_hbm, wqa_hbm, woa_hbm, wqb_hbm, wob_hbm, out_hbm,
            xres, xio, wq, wo, ws, q_s, k_s, v_s, o_s, xn_s, sems):
    f32, bf16, i32 = jnp.float32, jnp.bfloat16, jnp.int32

    cp_x0 = pltpu.make_async_copy(x_hbm.at[0:2 * R], xio.at[0:2 * R], sems.at[0])
    cp_x1 = pltpu.make_async_copy(x_hbm.at[2 * R:S], xio.at[2 * R:S], sems.at[1])
    cp_woa = pltpu.make_async_copy(woa_hbm, wo.at[0], sems.at[2])
    cp_wqb = pltpu.make_async_copy(wqb_hbm, wq.at[1], sems.at[3])
    cp_wob = pltpu.make_async_copy(wob_hbm, wo.at[1], sems.at[4])

    def cp_wqa(u):
        c = (u % 3) * D + (u // 3) * 128
        return [pltpu.make_async_copy(wqa_hbm.at[:, pl.ds(c + h * HD, 128)],
                                      wq.at[0, :, pl.ds(c + h * HD, 128)],
                                      sems.at[6 + u]) for h in range(2)]

    cp_x0.start()
    for u in range(3):
        for cp in cp_wqa(u):
            cp.start()

    k_s[:, PAD - 32:PAD, :] = jnp.zeros((NG, 32, 128), bf16)
    v_s[:, PAD - 32:PAD, :] = jnp.zeros((NG, 32, 128), bf16)

    def cvt(i, c):
        r0 = pl.multiple_of(i * R, R)
        xres[pl.ds(r0, R), :] = xio[pl.ds(r0, R), :].astype(f32)
        return c

    def lane_group(n):
        return lax.broadcasted_iota(i32, (n, 128), 1) // DH

    def stack_heads(q):
        n = q.shape[0]
        qi = pltpu.bitcast(q, i32)
        lg = lane_group(n // 2)
        parts = [pltpu.bitcast(jnp.where(lg == h, qi, 0), bf16) for h in range(4)]
        return jnp.concatenate(parts, axis=0)

    def prep_weights(raw, c0, dst):
        ch = 64
        for r0 in range(0, HD, ch):
            def ld(r, c):
                return raw[r * HD + r0:r * HD + r0 + ch,
                           pl.ds(pl.multiple_of(c0 + c * HD, 128), 128)]
            b11, b12, b21, b22 = ld(0, 0), ld(0, 1), ld(1, 0), ld(1, 1)
            w11, w12, w21, w22 = (b.astype(f32) for b in (b11, b12, b21, b22))
            rows = slice(r0, r0 + ch)
            dst[0, rows] = (w11 + w22).astype(bf16)
            dst[1, rows] = b11
            dst[2, rows] = (w12 - w22).astype(bf16)
            dst[3, rows] = (w21 - w11).astype(bf16)
            dst[4, rows] = b22
            dst[5, rows] = (w11 + w12).astype(bf16)
            dst[6, rows] = (w21 + w22).astype(bf16)

    def prep_qkv(wi, which, pi_):
        prep_weights(wq.at[wi], which * D + pi_ * 128, ws.at[wi, which * 4 + pi_])

    def prep_out(wi, pi_):
        prep_weights(wo.at[wi], pi_ * 128, ws.at[wi, 12 + pi_])

    def strassen(lhs, rhs):
        def mm(i):
            return jnp.dot(lhs[i], rhs[i], preferred_element_type=f32)
        m1 = mm(0)
        m2 = mm(1)
        c22 = m1 - m2
        m4 = mm(3)
        c21 = m2 + m4
        c11 = m1 + m4
        m3 = mm(2)
        c22 = c22 + m3
        m5 = mm(4)
        c12 = m3 + m5
        c11 = c11 - m5
        c22 = c22 + mm(5)
        c11 = c11 + mm(6)
        return c11, c12, c21, c22

    def part_ln(blk, r):
        r16 = pl.multiple_of(r * 16, 16)

        def ln(off):
            x = xres[pl.ds(pl.multiple_of(blk * R + off + r16, 16), 16), :]
            m = jnp.mean(x, axis=-1, keepdims=True)
            xc = x - m
            v = jnp.mean(xc * xc, axis=-1, keepdims=True)
            return xc * lax.rsqrt(v + EPS)
        top, bot = ln(0), ln(R // 2)
        for i, l in enumerate(_strassen_lhs(top[:, :HD], top[:, HD:], bot[:, :HD], bot[:, HD:])):
            xn_s[blk % 2, i, pl.ds(r16, 16), :] = l.astype(bf16)

    def part_qkv(wi, blk, pi_, whichs=(0, 1, 2)):
        r0 = pl.multiple_of(blk * R, R)
        for which in whichs:
            cs = strassen(xn_s.at[blk % 2], ws.at[wi, which * 4 + pi_])
            for n, c in enumerate(cs):
                g = pi_ + 4 * (n % 2)
                rr = r0 + (n // 2) * (R // 2)
                if which == 0:
                    q_s[g, pl.ds(rr, R // 2), :] = (c * QSCALE).astype(bf16)
                elif which == 1:
                    k_s[g, pl.ds(rr + PAD, R // 2), :] = c.astype(bf16)
                else:
                    v_s[g, pl.ds(rr + PAD, R // 2), :] = c.astype(bf16)

    def part_out(wi, blk, pi_, last):
        r0 = pl.multiple_of(blk * R, R)
        cs = strassen(o_s.at[blk % 2], ws.at[wi, 12 + pi_])
        for n, c in enumerate(cs):
            c0 = pl.multiple_of(pi_ * 128 + HD * (n % 2), 128)
            rr = r0 + (n // 2) * (R // 2)
            y = c + xres[pl.ds(rr, R // 2), pl.ds(c0, 128)]
            if last:
                xio[pl.ds(rr, R // 2), pl.ds(c0, 128)] = y.astype(bf16)
            else:
                xres[pl.ds(rr, R // 2), pl.ds(c0, 128)] = y

    def store_o(blk, pi_, oa, ob):
        c0 = pl.multiple_of(pi_ * 128, 128)
        h = R // 2
        for i, l in enumerate(_strassen_lhs(oa[:h], ob[:h], oa[h:], ob[h:])):
            o_s[blk % 2, i, :, pl.ds(c0, 128)] = l.astype(bf16)

    def seg_reduce(x, op, fill):
        lg = lane_group(x.shape[0])
        r = None
        for h in range(4):
            rh = op(jnp.where(lg == h, x, fill), axis=-1, keepdims=True)
            r = jnp.broadcast_to(rh, x.shape) if r is None else jnp.where(lg == h, rh, r)
        return r

    def tri_mask(n):
        kk = lax.broadcasted_iota(i32, (n, 128), 1) % DH
        return kk <= lax.broadcasted_iota(i32, (n, 128), 0)

    def tri_mask_packed(n):
        kk = lax.broadcasted_iota(i32, (n // 2, 128), 1) % DH
        row2 = lax.broadcasted_iota(i32, (n // 2, 128), 0) * 2
        return jnp.where(kk <= row2, 0x0000FFFF, 0) | jnp.where(kk <= row2 + 1, -65536, 0)

    def a_load(g, blk, edge):
        r0 = pl.multiple_of(blk * R, R)
        k0 = 8 if edge else 0
        w = pl.ds(r0 + 32 * k0, 32 * (16 - k0))
        return q_s[g, pl.ds(r0, R), :], k_s[g, w, :], v_s[g, w, :]

    def a_scores(q, kw, edge):
        k0 = 8 if edge else 0
        ss = {}
        for kb in range(k0, 16):
            kbd = stack_heads(kw[32 * (kb - k0):32 * (kb - k0) + 32])
            qq = q[0:32 * kb + 32] if kb < 8 else q[32 * (kb - 8):R]
            ss[kb] = lax.dot_general(qq, kbd, _NT, preferred_element_type=f32)
        return ss

    def a_softmax(ss, edge):
        tri = tri_mask(32)
        t = {}
        for kb in range(8):
            for rb in range(8):
                if rb == kb:
                    old = NEG if edge else ss[kb][32 * kb:32 * kb + 32]
                    t[kb, rb] = jnp.where(tri, ss[kb + 8][0:32], old)
                elif rb > kb:
                    t[kb, rb] = ss[kb + 8][32 * (rb - kb):32 * (rb - kb) + 32]
                elif not edge:
                    t[kb, rb] = ss[kb][32 * rb:32 * rb + 32]
        trip = tri_mask_packed(32)
        pp, rl = {}, []
        for rb in range(8):
            ks = [kb for kb in range(8) if (kb, rb) in t]
            m = functools.reduce(jnp.maximum, [t[kb, rb] for kb in ks])
            m = seg_reduce(m, jnp.max, -jnp.inf)
            p = {kb: jnp.exp2(t[kb, rb] - m) for kb in ks}
            l = seg_reduce(functools.reduce(jnp.add, [p[kb] for kb in ks]), jnp.sum, 0.0)
            rl.append(1.0 / l)
            for kb in ks:
                pb = p[kb].astype(bf16)
                if kb == rb:
                    pi = pltpu.bitcast(pb, i32)
                    pp[kb + 8, rb] = pltpu.bitcast(pi & trip, bf16)
                    if not edge:
                        pp[kb, rb] = pltpu.bitcast(pi & (~trip), bf16)
                elif rb > kb:
                    pp[kb + 8, rb] = pb
                else:
                    pp[kb, rb] = pb
        return pp, rl

    def a_values(edge, vw, pp, rl):
        k0 = 8 if edge else 0
        acc = [None] * 8
        for kb in range(k0, 16):
            vbd = stack_heads(vw[32 * (kb - k0):32 * (kb - k0) + 32])
            rbs = list(range(0, kb + 1)) if kb < 8 else list(range(kb - 8, 8))
            p = jnp.concatenate([pp[kb, rb] for rb in rbs], axis=0)
            o = jnp.dot(p, vbd, preferred_element_type=f32)
            for n, rb in enumerate(rbs):
                ob = o[32 * n:32 * n + 32]
                acc[rb] = ob if acc[rb] is None else acc[rb] + ob
        return jnp.concatenate([acc[rb] * rl[rb] for rb in range(8)], axis=0)

    def b_load(g, blk):
        r0 = pl.multiple_of(blk * R, R)
        w = pl.ds(r0 + (PAD - 32), R + 32)
        return q_s[g, pl.ds(r0, R), :], k_s[g, w, :], v_s[g, w, :]

    def b_scores(q, kw):
        ss = {}
        for kb in range(-1, 8):
            kbd = stack_heads(kw[32 * (kb + 1):32 * (kb + 2)])
            qq = q[0:16] if kb < 0 else q[32 * kb:min(32 * kb + 48, R)]
            ss[kb] = lax.dot_general(qq, kbd, _NT, preferred_element_type=f32)
        return ss

    def b_softmax(ss, blk):
        tri = tri_mask(16)
        kk = lax.broadcasted_iota(i32, (32, 128), 1) % DH
        row = lax.broadcasted_iota(i32, (32, 128), 0)
        dl = (row - kk) & 31
        ok = (dl <= 14) & ((dl & 1) == 0)
        tiles = []
        for rb in range(8):
            prev = ss[-1] if rb == 0 else ss[rb - 1][32:48]
            top = jnp.where(tri, ss[rb][0:16], prev)
            tile = jnp.concatenate([top, ss[rb][16:32]], axis=0)
            okr = ok & ((kk <= row) | (blk > 0)) if rb == 0 else ok
            tiles.append(jnp.where(okr, tile, NEG))
        s = jnp.concatenate(tiles, axis=0)
        m = seg_reduce(s, jnp.max, -jnp.inf)
        p = jnp.exp2(s - m)
        rl = 1.0 / seg_reduce(p, jnp.sum, 0.0)
        pb = p.astype(bf16)
        trip = tri_mask_packed(16)
        own, prv = [], []
        for rb in range(8):
            pi = pltpu.bitcast(pb[32 * rb:32 * rb + 16], i32)
            own.append(jnp.concatenate(
                [pltpu.bitcast(pi & trip, bf16), pb[32 * rb + 16:32 * rb + 32]], axis=0))
            prv.append(pltpu.bitcast(pi & (~trip), bf16))
        return own, prv, rl

    def b_values(vw, own, prv, rl):
        outs = {}
        for kb in range(-1, 8):
            vbd = stack_heads(vw[32 * (kb + 1):32 * (kb + 2)])
            if kb < 0:
                p = prv[0]
            elif kb < 7:
                p = jnp.concatenate([own[kb], prv[kb + 1]], axis=0)
            else:
                p = own[kb]
            outs[kb] = jnp.dot(p, vbd, preferred_element_type=f32)
        res = []
        for rb in range(8):
            prev = outs[-1] if rb == 0 else outs[rb - 1][32:48]
            o = jnp.concatenate([outs[rb][0:16] + prev, outs[rb][16:32]], axis=0)
            res.append(o)
        return jnp.concatenate(res, axis=0) * rl

    def out_dma(blk):
        r0 = pl.multiple_of(blk * R, R)
        return pltpu.make_async_copy(xio.at[pl.ds(r0, R), :], out_hbm.at[pl.ds(r0, R), :],
                                     sems.at[5])

    def run_steps(typ, pair, i_lo, i_hi, edge=False, tail=False):
        nc = NG // 2

        def body(t, c):
            i = i_lo + t // nc
            pi_ = t % nc
            gs = [pi_, pi_ + 4]
            qkv = [a_load(g, i, edge) if typ == 0 else b_load(g, i) for g in gs]
            final = pair == 1 and typ == 1
            ps, os_ = {}, {}

            def score(n):
                q, kw, _ = qkv[n]
                if typ == 0:
                    ps[n] = a_softmax(a_scores(q, kw, edge), edge)
                else:
                    ps[n] = b_softmax(b_scores(q, kw), i)

            def value(n):
                if typ == 0:
                    os_[n] = a_values(edge, qkv[n][2], *ps[n])
                else:
                    os_[n] = b_values(qkv[n][2], *ps[n])
                if len(os_) == 2:
                    store_o(i, pi_, os_[0], os_[1])

            def out():
                if edge and pair == 0:
                    return
                if i_lo >= 1:
                    part_out(typ, i - 1, pi_, final)
                else:
                    part_out((typ + NB + (i - 1) // NB) % 2, (i + NB - 1) % NB, pi_, False)

            def ln():
                if not tail:
                    for u in range(2):
                        part_ln((i + 2) % NB, 2 * pi_ + u)

            for op in ORDER[typ]:
                if op[0] == "s":
                    score(int(op[1]))
                elif op[0] == "v":
                    value(int(op[1]))
                elif op[0] == "o":
                    out()
                elif op[0] == "l":
                    ln()
                elif not tail:
                    part_qkv((typ + (i + 1) // NB) % 2, (i + 1) % NB, pi_, (int(op[1]),))
            if final and i_lo >= 1:
                @pl.when(pi_ == nc - 1)
                def _():
                    out_dma(i - 1).start()
            return c
        lax.fori_loop(0, (i_hi - i_lo) * nc, body, 0)

    cp_x0.wait()
    lax.fori_loop(0, 2, cvt, 0)

    def pro_ln(t, c):
        for r in range(NG):
            part_ln(t, r)
        return c
    lax.fori_loop(0, 2, pro_ln, 0)

    def fetch(u):
        for cp in cp_wqa(u):
            cp.wait()
        if u + 3 < 12:
            for cp in cp_wqa(u + 3):
                cp.start()
        if u == 7:
            cp_x1.start()
        if u == 10:
            cp_woa.start()
        if u == 11:
            cp_wqb.start()
            cp_wob.start()
        prep_qkv(0, u % 3, u // 3)

    fetch(0)
    for u in range(12):
        if u + 1 < 12:
            fetch(u + 1)
        part_qkv(0, 0, u // 3, (u % 3,))
    cp_x1.wait()
    lax.fori_loop(2, NB, cvt, 0)

    def prep_loop(fn, n):
        def body(t, c):
            fn(t)
            return c
        lax.fori_loop(0, n, body, 0)

    for pair in range(2):
        run_steps(0, pair, 0, 1, edge=True)
        if pair == 0:
            cp_woa.wait()
            prep_loop(lambda t: prep_out(0, t), 4)
            run_steps(0, pair, 1, 4)
            cp_wqb.wait()
            cp_wob.wait()
            for which in range(3):
                prep_loop(lambda t: prep_qkv(1, which, t), 4)
            prep_loop(lambda t: prep_out(1, t), 4)
            run_steps(0, pair, 4, NB)
            run_steps(1, pair, 0, NB)
        else:
            run_steps(0, pair, 1, NB)
            run_steps(1, pair, 0, 1)
            run_steps(1, pair, 1, NB - 1)
            run_steps(1, pair, NB - 1, NB, tail=True)

    def epi(t, c):
        part_out(1, NB - 1, t, True)
        return c
    lax.fori_loop(0, 4, epi, 0)
    out_dma(NB - 1).start()
    pltpu.make_async_copy(xio, out_hbm, sems.at[5]).wait()


@jax.jit
def pallas_interleave_layers__sliding_block__sliding_local_dilated__prompt_kernel(
    A_x: jax.Array,
    A_wqkv: jax.Array,
    A_wo: jax.Array,
    B_x: jax.Array,
    B_wqkv: jax.Array,
    B_wo: jax.Array,
):
    del B_x
    bf16, f32 = jnp.bfloat16, jnp.float32
    any_spec = pl.BlockSpec(memory_space=pl.ANY)
    out = pl.pallas_call(
        _kernel,
        in_specs=[any_spec] * 5,
        out_specs=any_spec,
        out_shape=jax.ShapeDtypeStruct((S, D), bf16),
        scratch_shapes=[
            pltpu.VMEM((S, D), f32),
            pltpu.VMEM((S, D), bf16),
            pltpu.VMEM((2, D, 3 * D), bf16),
            pltpu.VMEM((2, D, D), bf16),
            pltpu.VMEM((2, 16, 7, HD, 128), bf16),
            pltpu.VMEM((NG, S, 128), bf16),
            pltpu.VMEM((NG, PAD + S, 128), bf16),
            pltpu.VMEM((NG, PAD + S, 128), bf16),
            pltpu.VMEM((2, 7, R // 2, HD), bf16),
            pltpu.VMEM((2, 7, R // 2, HD), bf16),
            pltpu.SemaphoreType.DMA((18,)),
        ],
        compiler_params=pltpu.CompilerParams(vmem_limit_bytes=100 * 1024 * 1024),
    )(A_x.reshape(S, D), A_wqkv, A_wo, B_wqkv, B_wo)
    return out.reshape(1, S, D)
```

```python
import functools
import math

import jax
import jax.numpy as jnp
from jax import lax
import jax.experimental.pallas as pl
import jax.experimental.pallas.tpu as pltpu

S = 2048
D = 1024
NG = 8
DH = 32
PAD = 256
R = 256
NB = S // R
ORDER = ("s0 l o s1 p0 p1 v0 v1 p2".split(), "s0 l o s1 p0 p1 v0 p2 v1".split())
HD = D // 2
EPS = 1e-5
NEG = -1e9
QSCALE = (DH ** -0.5) * math.log2(math.e)

_NT = (((1,), (1,)), ((), ()))


def _strassen_lhs(x11, x12, x21, x22):
    return (x11 + x22, x21 + x22, x11, x22, x11 + x12, x21 - x11, x12 - x22)


def _kernel(x_hbm, wqa_hbm, woa_hbm, wqb_hbm, wob_hbm, out_hbm,
            xres, xio, wq, wo, ws, q_s, k_s, v_s, o_s, xn_s, sems):
    f32, bf16, i32 = jnp.float32, jnp.bfloat16, jnp.int32

    cp_x0 = pltpu.make_async_copy(x_hbm.at[0:2 * R], xio.at[0:2 * R], sems.at[0])
    cp_x1 = pltpu.make_async_copy(x_hbm.at[2 * R:S], xio.at[2 * R:S], sems.at[1])
    cp_woa = pltpu.make_async_copy(woa_hbm, wo.at[0], sems.at[2])
    cp_wqb = pltpu.make_async_copy(wqb_hbm, wq.at[1], sems.at[3])
    cp_wob = pltpu.make_async_copy(wob_hbm, wo.at[1], sems.at[4])

    def cp_wqa(u):
        c = (u % 3) * D + (u // 3) * 128
        return [pltpu.make_async_copy(wqa_hbm.at[:, pl.ds(c + h * HD, 128)],
                                      wq.at[0, :, pl.ds(c + h * HD, 128)],
                                      sems.at[6 + u]) for h in range(2)]

    cp_x0.start()
    for u in range(4):
        for cp in cp_wqa(u):
            cp.start()

    k_s[:, PAD - 32:PAD, :] = jnp.zeros((NG, 32, 128), bf16)
    v_s[:, PAD - 32:PAD, :] = jnp.zeros((NG, 32, 128), bf16)

    def cvt(i, c):
        r0 = pl.multiple_of(i * R, R)
        xres[pl.ds(r0, R), :] = xio[pl.ds(r0, R), :].astype(f32)
        return c

    def lane_group(n):
        return lax.broadcasted_iota(i32, (n, 128), 1) // DH

    def stack_heads(q):
        n = q.shape[0]
        qi = pltpu.bitcast(q, i32)
        lg = lane_group(n // 2)
        parts = [pltpu.bitcast(jnp.where(lg == h, qi, 0), bf16) for h in range(4)]
        return jnp.concatenate(parts, axis=0)

    def prep_weights(raw, c0, dst):
        ch = 64
        for r0 in range(0, HD, ch):
            def ld(r, c):
                return raw[r * HD + r0:r * HD + r0 + ch,
                           pl.ds(pl.multiple_of(c0 + c * HD, 128), 128)]
            b11, b12, b21, b22 = ld(0, 0), ld(0, 1), ld(1, 0), ld(1, 1)
            w11, w12, w21, w22 = (b.astype(f32) for b in (b11, b12, b21, b22))
            rows = slice(r0, r0 + ch)
            dst[0, rows] = (w11 + w22).astype(bf16)
            dst[1, rows] = b11
            dst[2, rows] = (w12 - w22).astype(bf16)
            dst[3, rows] = (w21 - w11).astype(bf16)
            dst[4, rows] = b22
            dst[5, rows] = (w11 + w12).astype(bf16)
            dst[6, rows] = (w21 + w22).astype(bf16)

    def prep_qkv(wi, which, pi_):
        prep_weights(wq.at[wi], which * D + pi_ * 128, ws.at[wi, which * 4 + pi_])

    def prep_out(wi, pi_):
        prep_weights(wo.at[wi], pi_ * 128, ws.at[wi, 12 + pi_])

    def strassen(lhs, rhs):
        def mm(i):
            return jnp.dot(lhs[i], rhs[i], preferred_element_type=f32)
        m1 = mm(0)
        m2 = mm(1)
        c22 = m1 - m2
        m4 = mm(3)
        c21 = m2 + m4
        c11 = m1 + m4
        m3 = mm(2)
        c22 = c22 + m3
        m5 = mm(4)
        c12 = m3 + m5
        c11 = c11 - m5
        c22 = c22 + mm(5)
        c11 = c11 + mm(6)
        return c11, c12, c21, c22

    def part_ln(blk, r):
        r16 = pl.multiple_of(r * 16, 16)

        def ln(off):
            x = xres[pl.ds(pl.multiple_of(blk * R + off + r16, 16), 16), :]
            m = jnp.mean(x, axis=-1, keepdims=True)
            xc = x - m
            v = jnp.mean(xc * xc, axis=-1, keepdims=True)
            return xc * lax.rsqrt(v + EPS)
        top, bot = ln(0), ln(R // 2)
        for i, l in enumerate(_strassen_lhs(top[:, :HD], top[:, HD:], bot[:, :HD], bot[:, HD:])):
            xn_s[blk % 2, i, pl.ds(r16, 16), :] = l.astype(bf16)

    def part_qkv(wi, blk, pi_, whichs=(0, 1, 2)):
        r0 = pl.multiple_of(blk * R, R)
        for which in whichs:
            cs = strassen(xn_s.at[blk % 2], ws.at[wi, which * 4 + pi_])
            for n, c in enumerate(cs):
                g = pi_ + 4 * (n % 2)
                rr = r0 + (n // 2) * (R // 2)
                if which == 0:
                    q_s[g, pl.ds(rr, R // 2), :] = (c * QSCALE).astype(bf16)
                elif which == 1:
                    k_s[g, pl.ds(rr + PAD, R // 2), :] = c.astype(bf16)
                else:
                    v_s[g, pl.ds(rr + PAD, R // 2), :] = c.astype(bf16)

    def part_out(wi, blk, pi_, last):
        r0 = pl.multiple_of(blk * R, R)
        cs = strassen(o_s.at[blk % 2], ws.at[wi, 12 + pi_])
        for n, c in enumerate(cs):
            c0 = pl.multiple_of(pi_ * 128 + HD * (n % 2), 128)
            rr = r0 + (n // 2) * (R // 2)
            y = c + xres[pl.ds(rr, R // 2), pl.ds(c0, 128)]
            if last:
                xio[pl.ds(rr, R // 2), pl.ds(c0, 128)] = y.astype(bf16)
            else:
                xres[pl.ds(rr, R // 2), pl.ds(c0, 128)] = y

    def store_o(blk, pi_, oa, ob):
        c0 = pl.multiple_of(pi_ * 128, 128)
        h = R // 2
        for i, l in enumerate(_strassen_lhs(oa[:h], ob[:h], oa[h:], ob[h:])):
            o_s[blk % 2, i, :, pl.ds(c0, 128)] = l.astype(bf16)

    def seg_reduce(x, op, fill):
        lg = lane_group(x.shape[0])
        r = None
        for h in range(4):
            rh = op(jnp.where(lg == h, x, fill), axis=-1, keepdims=True)
            r = jnp.broadcast_to(rh, x.shape) if r is None else jnp.where(lg == h, rh, r)
        return r

    def tri_mask(n):
        kk = lax.broadcasted_iota(i32, (n, 128), 1) % DH
        return kk <= lax.broadcasted_iota(i32, (n, 128), 0)

    def tri_mask_packed(n):
        kk = lax.broadcasted_iota(i32, (n // 2, 128), 1) % DH
        row2 = lax.broadcasted_iota(i32, (n // 2, 128), 0) * 2
        return jnp.where(kk <= row2, 0x0000FFFF, 0) | jnp.where(kk <= row2 + 1, -65536, 0)

    def a_load(g, blk, edge):
        r0 = pl.multiple_of(blk * R, R)
        k0 = 8 if edge else 0
        w = pl.ds(r0 + 32 * k0, 32 * (16 - k0))
        return q_s[g, pl.ds(r0, R), :], k_s[g, w, :], v_s[g, w, :]

    def a_scores(q, kw, edge):
        k0 = 8 if edge else 0
        ss = {}
        for kb in range(k0, 16):
            kbd = stack_heads(kw[32 * (kb - k0):32 * (kb - k0) + 32])
            qq = q[0:32 * kb + 32] if kb < 8 else q[32 * (kb - 8):R]
            ss[kb] = lax.dot_general(qq, kbd, _NT, preferred_element_type=f32)
        return ss

    def a_softmax(ss, edge):
        tri = tri_mask(32)
        t = {}
        for kb in range(8):
            for rb in range(8):
                if rb == kb:
                    old = NEG if edge else ss[kb][32 * kb:32 * kb + 32]
                    t[kb, rb] = jnp.where(tri, ss[kb + 8][0:32], old)
                elif rb > kb:
                    t[kb, rb] = ss[kb + 8][32 * (rb - kb):32 * (rb - kb) + 32]
                elif not edge:
                    t[kb, rb] = ss[kb][32 * rb:32 * rb + 32]
        trip = tri_mask_packed(32)
        pp, rl = {}, []
        for rb in range(8):
            ks = [kb for kb in range(8) if (kb, rb) in t]
            m = functools.reduce(jnp.maximum, [t[kb, rb] for kb in ks])
            m = seg_reduce(m, jnp.max, -jnp.inf)
            p = {kb: jnp.exp2(t[kb, rb] - m) for kb in ks}
            l = seg_reduce(functools.reduce(jnp.add, [p[kb] for kb in ks]), jnp.sum, 0.0)
            rl.append(1.0 / l)
            for kb in ks:
                pb = p[kb].astype(bf16)
                if kb == rb:
                    pi = pltpu.bitcast(pb, i32)
                    pp[kb + 8, rb] = pltpu.bitcast(pi & trip, bf16)
                    if not edge:
                        pp[kb, rb] = pltpu.bitcast(pi & (~trip), bf16)
                elif rb > kb:
                    pp[kb + 8, rb] = pb
                else:
                    pp[kb, rb] = pb
        return pp, rl

    def a_values(edge, vw, pp, rl):
        k0 = 8 if edge else 0
        acc = [None] * 8
        for kb in range(k0, 16):
            vbd = stack_heads(vw[32 * (kb - k0):32 * (kb - k0) + 32])
            rbs = list(range(0, kb + 1)) if kb < 8 else list(range(kb - 8, 8))
            p = jnp.concatenate([pp[kb, rb] for rb in rbs], axis=0)
            o = jnp.dot(p, vbd, preferred_element_type=f32)
            for n, rb in enumerate(rbs):
                ob = o[32 * n:32 * n + 32]
                acc[rb] = ob if acc[rb] is None else acc[rb] + ob
        return jnp.concatenate([acc[rb] * rl[rb] for rb in range(8)], axis=0)

    def b_load(g, blk):
        r0 = pl.multiple_of(blk * R, R)
        w = pl.ds(r0 + (PAD - 32), R + 32)
        return q_s[g, pl.ds(r0, R), :], k_s[g, w, :], v_s[g, w, :]

    def b_scores(q, kw):
        ss = {}
        for kb in range(-1, 8):
            kbd = stack_heads(kw[32 * (kb + 1):32 * (kb + 2)])
            qq = q[0:16] if kb < 0 else q[32 * kb:min(32 * kb + 48, R)]
            ss[kb] = lax.dot_general(qq, kbd, _NT, preferred_element_type=f32)
        return ss

    def b_softmax(ss, blk):
        tri = tri_mask(16)
        kk = lax.broadcasted_iota(i32, (32, 128), 1) % DH
        row = lax.broadcasted_iota(i32, (32, 128), 0)
        dl = (row - kk) & 31
        ok = (dl <= 14) & ((dl & 1) == 0)
        tiles = []
        for rb in range(8):
            prev = ss[-1] if rb == 0 else ss[rb - 1][32:48]
            top = jnp.where(tri, ss[rb][0:16], prev)
            tile = jnp.concatenate([top, ss[rb][16:32]], axis=0)
            okr = ok & ((kk <= row) | (blk > 0)) if rb == 0 else ok
            tiles.append(jnp.where(okr, tile, NEG))
        s = jnp.concatenate(tiles, axis=0)
        m = seg_reduce(s, jnp.max, -jnp.inf)
        p = jnp.exp2(s - m)
        rl = 1.0 / seg_reduce(p, jnp.sum, 0.0)
        pb = p.astype(bf16)
        trip = tri_mask_packed(16)
        own, prv = [], []
        for rb in range(8):
            pi = pltpu.bitcast(pb[32 * rb:32 * rb + 16], i32)
            own.append(jnp.concatenate(
                [pltpu.bitcast(pi & trip, bf16), pb[32 * rb + 16:32 * rb + 32]], axis=0))
            prv.append(pltpu.bitcast(pi & (~trip), bf16))
        return own, prv, rl

    def b_values(vw, own, prv, rl):
        outs = {}
        for kb in range(-1, 8):
            vbd = stack_heads(vw[32 * (kb + 1):32 * (kb + 2)])
            if kb < 0:
                p = prv[0]
            elif kb < 7:
                p = jnp.concatenate([own[kb], prv[kb + 1]], axis=0)
            else:
                p = own[kb]
            outs[kb] = jnp.dot(p, vbd, preferred_element_type=f32)
        res = []
        for rb in range(8):
            prev = outs[-1] if rb == 0 else outs[rb - 1][32:48]
            o = jnp.concatenate([outs[rb][0:16] + prev, outs[rb][16:32]], axis=0)
            res.append(o)
        return jnp.concatenate(res, axis=0) * rl

    def out_dma(blk):
        r0 = pl.multiple_of(blk * R, R)
        return pltpu.make_async_copy(xio.at[pl.ds(r0, R), :], out_hbm.at[pl.ds(r0, R), :],
                                     sems.at[5])

    def run_steps(typ, pair, i_lo, i_hi, edge=False, tail=False):
        nc = NG // 2

        def body(t, c):
            i = i_lo + t // nc
            pi_ = t % nc
            gs = [pi_, pi_ + 4]
            qkv = [a_load(g, i, edge) if typ == 0 else b_load(g, i) for g in gs]
            final = pair == 1 and typ == 1
            ps, os_ = {}, {}

            def score(n):
                q, kw, _ = qkv[n]
                if typ == 0:
                    ps[n] = a_softmax(a_scores(q, kw, edge), edge)
                else:
                    ps[n] = b_softmax(b_scores(q, kw), i)

            def value(n):
                if typ == 0:
                    os_[n] = a_values(edge, qkv[n][2], *ps[n])
                else:
                    os_[n] = b_values(qkv[n][2], *ps[n])
                if len(os_) == 2:
                    store_o(i, pi_, os_[0], os_[1])

            def out():
                if edge and pair == 0:
                    return
                if i_lo >= 1:
                    part_out(typ, i - 1, pi_, final)
                else:
                    part_out((typ + NB + (i - 1) // NB) % 2, (i + NB - 1) % NB, pi_, False)

            def ln():
                if not tail:
                    for u in range(2):
                        part_ln((i + 2) % NB, 2 * pi_ + u)

            for op in ORDER[typ]:
                if op[0] == "s":
                    score(int(op[1]))
                elif op[0] == "v":
                    value(int(op[1]))
                elif op[0] == "o":
                    out()
                elif op[0] == "l":
                    ln()
                elif not tail:
                    part_qkv((typ + (i + 1) // NB) % 2, (i + 1) % NB, pi_, (int(op[1]),))
            if final and i_lo >= 1:
                @pl.when(pi_ == nc - 1)
                def _():
                    out_dma(i - 1).start()
            return c
        lax.fori_loop(0, (i_hi - i_lo) * nc, body, 0)

    cp_x0.wait()
    lax.fori_loop(0, 2, cvt, 0)

    def pro_ln(t, c):
        for r in range(NG):
            part_ln(t, r)
        return c
    lax.fori_loop(0, 2, pro_ln, 0)

    def fetch(c):
        us = range(2 * c, 2 * c + 2)
        for u in us:
            for cp in cp_wqa(u):
                cp.wait()
        for u in us:
            if u + 4 < 12:
                for cp in cp_wqa(u + 4):
                    cp.start()
        if c == 3:
            cp_x1.start()
        if c == 4:
            cp_woa.start()
        if c == 5:
            cp_wqb.start()
            cp_wob.start()
        for u in us:
            prep_qkv(0, u % 3, u // 3)

    fetch(0)
    for c in range(6):
        if c + 1 < 6:
            fetch(c + 1)
        for u in range(2 * c, 2 * c + 2):
            part_qkv(0, 0, u // 3, (u % 3,))
    cp_x1.wait()
    lax.fori_loop(2, NB, cvt, 0)

    def prep_loop(fn, n):
        def body(t, c):
            fn(t)
            return c
        lax.fori_loop(0, n, body, 0)

    for pair in range(2):
        run_steps(0, pair, 0, 1, edge=True)
        if pair == 0:
            cp_woa.wait()
            prep_loop(lambda t: prep_out(0, t), 4)
            run_steps(0, pair, 1, 4)
            cp_wqb.wait()
            cp_wob.wait()
            for which in range(3):
                prep_loop(lambda t: prep_qkv(1, which, t), 4)
            prep_loop(lambda t: prep_out(1, t), 4)
            run_steps(0, pair, 4, NB)
            run_steps(1, pair, 0, NB)
        else:
            run_steps(0, pair, 1, NB)
            run_steps(1, pair, 0, 1)
            run_steps(1, pair, 1, NB - 1)
            run_steps(1, pair, NB - 1, NB, tail=True)

    def epi(t, c):
        part_out(1, NB - 1, t, True)
        return c
    lax.fori_loop(0, 4, epi, 0)
    out_dma(NB - 1).start()
    pltpu.make_async_copy(xio, out_hbm, sems.at[5]).wait()


@jax.jit
def pallas_interleave_layers__sliding_block__sliding_local_dilated__prompt_kernel(
    A_x: jax.Array,
    A_wqkv: jax.Array,
    A_wo: jax.Array,
    B_x: jax.Array,
    B_wqkv: jax.Array,
    B_wo: jax.Array,
):
    del B_x
    bf16, f32 = jnp.bfloat16, jnp.float32
    any_spec = pl.BlockSpec(memory_space=pl.ANY)
    out = pl.pallas_call(
        _kernel,
        in_specs=[any_spec] * 5,
        out_specs=any_spec,
        out_shape=jax.ShapeDtypeStruct((S, D), bf16),
        scratch_shapes=[
            pltpu.VMEM((S, D), f32),
            pltpu.VMEM((S, D), bf16),
            pltpu.VMEM((2, D, 3 * D), bf16),
            pltpu.VMEM((2, D, D), bf16),
            pltpu.VMEM((2, 16, 7, HD, 128), bf16),
            pltpu.VMEM((NG, S, 128), bf16),
            pltpu.VMEM((NG, PAD + S, 128), bf16),
            pltpu.VMEM((NG, PAD + S, 128), bf16),
            pltpu.VMEM((2, 7, R // 2, HD), bf16),
            pltpu.VMEM((2, 7, R // 2, HD), bf16),
            pltpu.SemaphoreType.DMA((18,)),
        ],
        compiler_params=pltpu.CompilerParams(vmem_limit_bytes=100 * 1024 * 1024),
    )(A_x.reshape(S, D), A_wqkv, A_wo, B_wqkv, B_wo)
    return out.reshape(1, S, D)
```
